```python
import os as _os
_os.environ.setdefault("JAX_PLATFORMS", "cpu")
import jax
import jax.numpy as jnp

def _softmax(x, axis=-1):
    return jax.nn.softmax(x, axis=axis)
def _gelu(x):
    return jax.nn.gelu(x, approximate=True)
def _silu(x):
    return jax.nn.silu(x)
def _sigmoid(x):
    return jax.nn.sigmoid(x)
def _layernorm(x, axis=-1, eps=1e-5):
    m = jnp.mean(x, axis=axis, keepdims=True)
    v = jnp.var(x, axis=axis, keepdims=True)
    return (x - m) / jnp.sqrt(v + eps)
def _scatter_add(tgt, idx, src, axis=0):
    return tgt.at[idx].add(src)
def _segment_sum(src, seg, n):
    return jax.ops.segment_sum(src, seg, n)
class _Rng:
    def __init__(self, key):
        self._k = key
    def _next(self):
        self._k, sub = jax.random.split(self._k)
        return sub
    def normal(self, shape):
        return jax.random.normal(self._next(), shape, dtype=jnp.bfloat16)
    def randint(self, lo, hi, shape):
        return jax.random.randint(self._next(), shape, lo, hi, dtype=jnp.int32)
    def uniform(self, shape, lo=0.0, hi=1.0):
        return jax.random.uniform(self._next(), shape, jnp.bfloat16, lo, hi)
    def permutation(self, n):
        return jax.random.permutation(self._next(), n)


kernel_name = 'standalone__geglu_ffn__prompt'

def setup_inputs():
    _rng = _Rng(jax.random.key(int.from_bytes(__import__("os").urandom(4), "little")))
    _w = (lambda a: (lambda t: t.astype(jnp.bfloat16) if jnp.issubdtype(t.dtype, jnp.floating) else t)(jnp.asarray(a)))
    B, S, D, F = 1, 2048, 576, 4608
    return {
        "x": _w((lambda *s: _rng.normal(s) * 0.05)(B, S, D)),
        "w_gate": _w((lambda *s: _rng.normal(s) * 0.05)(D, F)),
        "w_up": _w((lambda *s: _rng.normal(s) * 0.05)(D, F)),
        "w_down": _w((lambda *s: _rng.normal(s) * 0.05)(F, D)),
    }

def reference(x, w_gate, w_up, w_down):
    return (_gelu(x @ w_gate) * (x @ w_up)) @ w_down
```

```python
import functools

import jax
import jax.numpy as jnp
import jax.experimental.pallas as pl
import jax.experimental.pallas.tpu as pltpu


def _gelu_tanh(g):
    c = 0.7978845608028654
    inner = g * (c + (c * 0.044715) * (g * g))
    return 0.5 * g * (1.0 + jnp.tanh(inner))


def _kernel(x_ref, wg_ref, wu_ref, wd_ref, o_ref, acc_ref):
    f = pl.program_id(1)

    @pl.when(f == 0)
    def _():
        acc_ref[...] = jnp.zeros_like(acc_ref)

    x = x_ref[...]
    g = jnp.dot(x, wg_ref[...], preferred_element_type=jnp.float32)
    u = jnp.dot(x, wu_ref[...], preferred_element_type=jnp.float32)
    h = (_gelu_tanh(g) * u).astype(jnp.bfloat16)
    acc_ref[...] += jnp.dot(h, wd_ref[...], preferred_element_type=jnp.float32)

    @pl.when(f == pl.num_programs(1) - 1)
    def _():
        o_ref[...] = acc_ref[...].astype(o_ref.dtype)


@jax.jit
def pallas_standalone__geglu_ffn__prompt_kernel(
    x: jax.Array,
    w_gate: jax.Array,
    w_up: jax.Array,
    w_down: jax.Array,
):
    B, S, D = x.shape
    F = w_gate.shape[1]
    M = B * S
    x2 = x.reshape(M, D)
    tm, tf = 512, 512
    out = pl.pallas_call(
        _kernel,
        grid=(M // tm, F // tf),
        in_specs=[
            pl.BlockSpec((tm, D), lambda i, f: (i, 0)),
            pl.BlockSpec((D, tf), lambda i, f: (0, f)),
            pl.BlockSpec((D, tf), lambda i, f: (0, f)),
            pl.BlockSpec((tf, D), lambda i, f: (f, 0)),
        ],
        out_specs=pl.BlockSpec((tm, D), lambda i, f: (i, 0)),
        out_shape=jax.ShapeDtypeStruct((M, D), x.dtype),
        scratch_shapes=[pltpu.VMEM((tm, D), jnp.float32)],
        compiler_params=pltpu.CompilerParams(
            dimension_semantics=("parallel", "arbitrary"),
            vmem_limit_bytes=100 * 1024 * 1024,
        ),
    )(x2, w_gate, w_up, w_down)
    return out.reshape(B, S, D)
```

```python
import functools
import jax
import jax.numpy as jnp
from jax import lax
import jax.experimental.pallas as pl
import jax.experimental.pallas.tpu as pltpu

F32 = jnp.float32
BF16 = jnp.bfloat16
D, M, F = 576, 2048, 4608


def _act(g, u):
    c = 0.7978845608028654
    inner = g * (c + (c * 0.044715) * (g * g))
    return ((0.5 * g * (1.0 + jnp.tanh(inner))) * u).astype(BF16)


def _gu(x, wg, wu):
    g = jnp.dot(x, wg, preferred_element_type=F32)
    u = jnp.dot(x, wu, preferred_element_type=F32)
    return _act(g, u)


def _down(wdt, h):
    return lax.dot_general(wdt, h, (((1,), (1,)), ((), ())), preferred_element_type=F32)


def make(a=256, b=512, c=256, first=(256, 256, 512, 1024), last=(1024, 512, 256, 256), orows=1,
         mid=(2048,), nosem=True, splitgu=False):
    n = (F - a - c) // b
    assert a + n * b + c == F
    assert sum(first) == M and sum(last) == M and sum(mid) == M
    foff = [sum(first[:i]) for i in range(len(first))]
    loff = [sum(last[:i]) for i in range(len(last))]
    moff = [sum(mid[:i]) for i in range(len(mid))]
    NS, NL = len(first), len(last)

    def kern(xt_hbm, wg_hbm, wu_hbm, wd_hbm, o_hbm,
             xt_v, x_v, w0, wm, wl, acc, o_v, isem, osem):
        whbm = (wg_hbm, wu_hbm, wd_hbm)

        def xcp(s):
            sl = pl.ds(foff[s], first[s])
            return pltpu.make_async_copy(xt_hbm.at[:, sl], xt_v.at[:, sl], isem.at[s])

        def w0cp(w):
            return pltpu.make_async_copy(whbm[w].at[:, pl.ds(0, a)], w0.at[w], isem.at[NS + w])

        def wmcp(w, j):
            off = a + j * b
            if not isinstance(j, int):
                off = pl.multiple_of(off, 128)
            return pltpu.make_async_copy(whbm[w].at[:, pl.ds(off, b)], wm.at[w, j], isem.at[NS + 3 + j])

        def wlcp(w):
            return pltpu.make_async_copy(whbm[w].at[:, pl.ds(F - c, c)], wl.at[w], isem.at[NS + 3 + n])

        def ocp(s, r=0, nr=1):
            sl = pl.ds(loff[s], last[s])
            rs = pl.ds(r * (D // nr), D // nr)
            return pltpu.make_async_copy(o_v.at[rs, sl], o_hbm.at[rs, sl], osem.at[0])

        xcp(0).start()
        w0cp(0).start()
        w0cp(1).start()
        xcp(1).start()
        w0cp(2).start()
        for s in range(2, NS):
            xcp(s).start()
        for j in range(n):
            for w in range(3):
                wmcp(w, j).start(priority=1)
        for w in range(3):
            wlcp(w).start(priority=1)

        h_prev = None
        for s in range(NS):
            sl = pl.ds(foff[s], first[s])
            xcp(s).wait()
            if s == 1:
                w0cp(2).wait()
            x_v[sl, :] = xt_v[:, sl].T
            if s == 0:
                w0cp(0).wait()
                if splitgu:
                    g0 = jnp.dot(x_v[sl, :], w0[0], preferred_element_type=F32)
                w0cp(1).wait()
            if h_prev is not None:
                acc[:, pl.ds(foff[s - 1], first[s - 1])] = _down(w0[2], h_prev)
            if s == 0 and splitgu:
                h_prev = _act(g0, jnp.dot(x_v[sl, :], w0[1], preferred_element_type=F32))
            else:
                h_prev = _gu(x_v[sl, :], w0[0], w0[1])
        acc[:, pl.ds(foff[NS - 1], first[NS - 1])] = _down(w0[2], h_prev)

        def body(j, carry):
            for w in range(3):
                wmcp(w, j).wait()
            hp = None
            for s in range(len(mid)):
                h = _gu(x_v[pl.ds(moff[s], mid[s]), :], wm[0, j], wm[1, j])
                if hp is not None:
                    acc[:, pl.ds(moff[s - 1], mid[s - 1])] += _down(wm[2, j], hp)
                hp = h
            acc[:, pl.ds(moff[-1], mid[-1])] += _down(wm[2, j], hp)
            return carry

        lax.fori_loop(0, n, body, 0)

        for w in range(3):
            wlcp(w).wait()

        ocps = []

        def fin(s, h):
            sl = pl.ds(loff[s], last[s])
            nr = orows if s == NL - 1 else 1
            val = (acc[:, sl] + _down(wl[2], h)).astype(BF16)
            for r in range(nr):
                rs = pl.ds(r * (D // nr), D // nr)
                o_v[rs, sl] = val[r * (D // nr):(r + 1) * (D // nr)]
                cp = ocp(s, r, nr)
                cp.start()
                ocps.append(cp)

        h_prev = None
        for s in range(NL):
            sl = pl.ds(loff[s], last[s])
            h = _gu(x_v[sl, :], wl[0], wl[1])
            if h_prev is not None:
                fin(s - 1, h_prev)
            h_prev = h
        fin(NL - 1, h_prev)
        for cp in ocps:
            cp.wait()

    def fn(x, w_gate, w_up, w_down):
        B, S, _ = x.shape
        xt = x.reshape(M, D).T
        wdt = w_down.T
        out_t = pl.pallas_call(
            kern,
            in_specs=[pl.BlockSpec(memory_space=pl.ANY)] * 4,
            out_specs=pl.BlockSpec(memory_space=pl.ANY),
            out_shape=jax.ShapeDtypeStruct((D, M), x.dtype),
            scratch_shapes=[
                pltpu.VMEM((D, M), BF16),
                pltpu.VMEM((M, D), BF16),
                pltpu.VMEM((3, D, a), BF16),
                pltpu.VMEM((3, n, D, b), BF16),
                pltpu.VMEM((3, D, c), BF16),
                pltpu.VMEM((D, M), F32),
                pltpu.VMEM((D, M), BF16),
                pltpu.SemaphoreType.DMA((NS + 3 + n + 1,)),
                pltpu.SemaphoreType.DMA((1,)),
            ],
            compiler_params=pltpu.CompilerParams(vmem_limit_bytes=110 * 1024 * 1024,
                                                 disable_semaphore_checks=nosem),
        )(xt, w_gate, w_up, wdt)
        return out_t.T.reshape(B, S, D)
    return fn


_impl = make(splitgu=True)


@jax.jit
def pallas_standalone__geglu_ffn__prompt_kernel(
    x: jax.Array,
    w_gate: jax.Array,
    w_up: jax.Array,
    w_down: jax.Array,
):
    return _impl(x, w_gate, w_up, w_down)
```

```python
import jax
import jax.numpy as jnp
from jax import lax
import jax.experimental.pallas as pl
import jax.experimental.pallas.tpu as pltpu

F32 = jnp.float32
BF16 = jnp.bfloat16
U32 = jnp.uint32
D, M, F = 576, 2048, 4608
KM, KT = 512, 64


def _act(g, u):
    c = 0.7978845608028654
    inner = g * (c + (c * 0.044715) * (g * g))
    return ((0.5 * g * (1.0 + jnp.tanh(inner))) * u).astype(BF16)


def _dot(a, b):
    return jnp.dot(a, b, preferred_element_type=F32)


def _down(wdt, h):
    return lax.dot_general(wdt, h, (((1,), (1,)), ((), ())), preferred_element_type=F32)


def make(a=256, b=512, c=256, first=(256, 256, 512, 512, 512), last=(512, 512, 512, 256, 256), orows=4, nfin=2,
         mid=(512, 1536), TV=416, kq=(32, 32), scopes=False, xbs=2, tie=False, gt0=4, ut0=6):
    n = (F - a - c) // b
    assert a + n * b + c == F and c <= b
    assert sum(first) == M and sum(last) == M and sum(mid) == M
    assert TV <= mid[0] and TV <= last[0] and TV % 16 == 0
    foff = [sum(first[:i]) for i in range(len(first))]
    loff = [sum(last[:i]) for i in range(len(last))]
    moff = [sum(mid[:i]) for i in range(len(mid))]
    NS, NL = len(first), len(last)
    NT = b // 128
    NQ = len(kq)
    kqo = [sum(kq[:i]) for i in range(NQ + 1)]
    assert kqo[-1] == KT

    import contextlib
    scope = jax.named_scope if scopes else (lambda name: contextlib.nullcontext())

    def kern(xt_hbm, wg_hbm, wu_hbm, wd_hbm, o_hbm,
             xt_v, x32, w0, wm, wpk, acc, o_v, xb, w32, tt, zv, isem, osem):
        whbm = (wg_hbm, wu_hbm, wd_hbm)

        def xcp(s):
            sl = pl.ds(foff[s], first[s])
            return pltpu.make_async_copy(xt_hbm.at[:, sl], xt_v.at[:, sl], isem.at[s])

        def w0cp(w):
            return pltpu.make_async_copy(whbm[w].at[:, pl.ds(0, a)], w0.at[w], isem.at[NS + w])

        def wmcp(w, j):
            if isinstance(j, int):
                off = min(a + j * b, F - b)
            else:
                off = pl.multiple_of(jnp.minimum(a + j * b, F - b), 128)
            return pltpu.make_async_copy(whbm[w].at[:, pl.ds(off, b)], wm.at[w, j], isem.at[NS + 3 + j])

        def ocp(s, r, nr):
            sl = pl.ds(loff[s], last[s])
            rs = pl.ds(r * (D // nr), D // nr)
            return pltpu.make_async_copy(o_v.at[rs, sl], o_hbm.at[rs, sl], osem.at[0])

        def X(r0, nr, c0=0, nc=D):
            return pltpu.bitcast(x32[pl.ds(r0 // 2, nr // 2), pl.ds(c0, nc)], BF16)

        def WP(w, r0, nr, c0=0, nc=b):
            return pltpu.bitcast(wpk[w, pl.ds(r0 // 2, nr // 2), pl.ds(c0, nc)], BF16)

        def repack(j):
            for w in range(2):
                wpk[w] = pltpu.bitcast(wm[w, j], U32)

        xcp(0).start()
        w0cp(0).start()
        w0cp(1).start()
        xcp(1).start()
        w0cp(2).start()
        for s in range(2, NS):
            xcp(s).start()
        for j in range(n + 1):
            for w in range(3):
                wmcp(w, j).start(priority=1)

        zv[...] = jnp.zeros((8, 128), U32)
        for q in range(1, NQ):
            tt[q] = jnp.zeros((TV, 2 * b), F32)

        h_prev = None
        for s in range(NS):
          with scope(f"first{s}"):
            sl = pl.ds(foff[s], first[s])
            xcp(s).wait()
            if s == 1:
                w0cp(2).wait()
            if s == NS - 1:
                for w in range(3):
                    wmcp(w, 0).wait()
            x32[pl.ds(foff[s] // 2, first[s] // 2), :] = pltpu.bitcast(xt_v[:, sl].T, U32)
            if s == 0:
                w0cp(0).wait()
                g0 = _dot(X(foff[s], first[s]), w0[0])
                w0cp(1).wait()
            if h_prev is not None:
                acc[:, pl.ds(foff[s - 1], first[s - 1])] = _down(w0[2], h_prev)
            if s == 0:
                h_prev = _act(g0, _dot(X(foff[s], first[s]), w0[1]))
            else:
                xs = X(foff[s], first[s])
                h_prev = _act(_dot(xs, w0[0]), _dot(xs, w0[1]))
            if s >= xbs:
                ks = [k for k in range(KT) if k % (NS - xbs) == s - xbs]
                xtl = X(0, TV, KM, KT).astype(F32)
                for k in ks:
                    xb[k] = jnp.broadcast_to(xtl[:, k:k + 1], (TV, 128))
            if s == NS - 1:
                repack(0)
                xtl = X(0, TV, KM, KT)
                tt[0, :, pl.ds(0, b)] = _dot(xtl, wm[0, 0, pl.ds(KM, KT), :])
                tt[0, :, pl.ds(b, b)] = _dot(xtl, wm[1, 0, pl.ds(KM, KT), :])
                acc[:, pl.ds(foff[NS - 1], first[NS - 1])] = _down(w0[2], h_prev)

        def gu(r0, ts, tv, c0, nc):
            xm = X(r0, ts, 0, KM)
            g = _dot(xm, WP(0, 0, KM, c0, nc))
            u = _dot(xm, WP(1, 0, KM, c0, nc))
            pg, pu = [], []
            if tv:
                vg = tt[0, :, pl.ds(c0, nc)]
                vu = tt[0, :, pl.ds(b + c0, nc)]
                for q in range(1, NQ):
                    vg = vg + tt[q, :, pl.ds(c0, nc)]
                    vu = vu + tt[q, :, pl.ds(b + c0, nc)]
                pg.append(vg)
                pu.append(vu)
            if ts > tv:
                xt_ = X(r0 + tv, ts - tv, KM, KT)
                pg.append(_dot(xt_, WP(0, KM, KT, c0, nc)))
                pu.append(_dot(xt_, WP(1, KM, KT, c0, nc)))
            return _act(g + jnp.concatenate(pg, axis=0), u + jnp.concatenate(pu, axis=0))

        def body(j, carry):
            for w in range(3):
                wmcp(w, j + 1).wait()
            w32[:, pl.ds(0, b)] = wm[0, j + 1, pl.ds(KM, KT), :].astype(F32)
            w32[:, pl.ds(b, b)] = wm[1, j + 1, pl.ds(KM, KT), :].astype(F32)
            hs = [gu(moff[s], mid[s], TV if s == 0 else 0, 0, b) for s in range(len(mid))]
            items = {0: [(0, r, ci) for ci in range(NT) for r in range(D // 16)],
                     1: [(1, r, ci) for ci in range(NT) for r in range(D // 16)]}
            z = zv[...]
            for i in range(2 * NT):
                cs = pl.ds(i * 128, 128)
                for t0 in range(0, TV, 8):
                    rows = pl.ds(t0, 8)
                    for q in range(NQ):
                        r = None
                        if tie:
                            it = None
                            if i >= gt0 and items[0]:
                                it = items[0].pop(0)
                            elif i >= ut0 and items[1]:
                                it = items[1].pop(0)
                            if it is not None:
                                w, rr, ci = it
                                v = pltpu.bitcast(wm[w, j + 1, pl.ds(rr * 16, 16), pl.ds(ci * 128, 128)], U32)
                                wpk[w, pl.ds(rr * 8, 8), pl.ds(ci * 128, 128)] = v
                                r = pltpu.bitcast(v & z, F32)
                        for k in range(kqo[q], kqo[q + 1]):
                            p = xb[k, rows, :] * w32[pl.ds(k, 1), cs]
                            r = p if r is None else r + p
                        tt[q, rows, cs] = r
            for w in range(2):
                for (_, rr, ci) in items[w]:
                    wpk[w, pl.ds(rr * 8, 8), pl.ds(ci * 128, 128)] = pltpu.bitcast(
                        wm[w, j + 1, pl.ds(rr * 16, 16), pl.ds(ci * 128, 128)], U32)
            for s in range(len(mid)):
                acc[:, pl.ds(moff[s], mid[s])] += _down(wm[2, j], hs[s])
            return carry

        with scope("loop"):
            lax.fori_loop(0, n, body, 0)

        c0 = b - c
        ocps = []

        def fin(s, h):
            sl = pl.ds(loff[s], last[s])
            nr = orows if s >= NL - nfin else 1
            val = (acc[:, sl] + _down(wm[2, n, :, pl.ds(c0, c)], h)).astype(BF16)
            for r in range(nr):
                rs = pl.ds(r * (D // nr), D // nr)
                o_v[rs, sl] = val[r * (D // nr):(r + 1) * (D // nr)]
                cp = ocp(s, r, nr)
                cp.start()
                ocps.append(cp)

        h_prev = None
        for s in range(NL):
            h = gu(loff[s], last[s], TV if s == 0 else 0, c0, c)
            if h_prev is not None:
                fin(s - 1, h_prev)
            h_prev = h
        fin(NL - 1, h_prev)
        with scope("finalwait"):
            for cp in ocps:
                cp.wait()

    def fn(x, w_gate, w_up, w_down):
        B, S, _ = x.shape
        xt = x.reshape(M, D).T
        wdt = w_down.T
        out_t = pl.pallas_call(
            kern,
            in_specs=[pl.BlockSpec(memory_space=pl.ANY)] * 4,
            out_specs=pl.BlockSpec(memory_space=pl.ANY),
            out_shape=jax.ShapeDtypeStruct((D, M), x.dtype),
            scratch_shapes=[
                pltpu.VMEM((D, M), BF16),
                pltpu.VMEM((M // 2, D), U32),
                pltpu.VMEM((3, D, a), BF16),
                pltpu.VMEM((3, n + 1, D, b), BF16),
                pltpu.VMEM((2, D // 2, b), U32),
                pltpu.VMEM((D, M), F32),
                pltpu.VMEM((D, M), BF16),
                pltpu.VMEM((KT, TV, 128), F32),
                pltpu.VMEM((KT, 2 * b), F32),
                pltpu.VMEM((NQ, TV, 2 * b), F32),
                pltpu.VMEM((8, 128), U32),
                pltpu.SemaphoreType.DMA((NS + 3 + n + 1,)),
                pltpu.SemaphoreType.DMA((1,)),
            ],
            compiler_params=pltpu.CompilerParams(vmem_limit_bytes=110 * 1024 * 1024,
                                                 disable_semaphore_checks=True),
        )(xt, w_gate, w_up, wdt)
        return out_t.T.reshape(B, S, D)
    return fn


_impl = make()


@jax.jit
def pallas_standalone__geglu_ffn__prompt_kernel(
    x: jax.Array,
    w_gate: jax.Array,
    w_up: jax.Array,
    w_down: jax.Array,
):
    return _impl(x, w_gate, w_up, w_down)
```

```python
import jax
import jax.numpy as jnp
from jax import lax
import jax.experimental.pallas as pl
import jax.experimental.pallas.tpu as pltpu

F32 = jnp.float32
BF16 = jnp.bfloat16
U32 = jnp.uint32
D, M, F = 576, 2048, 4608
KM, KT = 512, 64


HALF = [True]


def _act(g, u):
    c = 0.7978845608028654
    inner = g * (c + (c * 0.044715) * (g * g))
    if HALF[0]:
        return ((0.5 * g * (1.0 + jnp.tanh(inner))) * u).astype(BF16)
    return ((g * (1.0 + jnp.tanh(inner))) * u).astype(BF16)


def _dot(a, b):
    return jnp.dot(a, b, preferred_element_type=F32)


def _down(wdt, h):
    return lax.dot_general(wdt, h, (((1,), (1,)), ((), ())), preferred_element_type=F32)


def make(a=256, b=512, c=256, first=(256, 256, 768, 768), last=(512, 512, 512, 256, 256), orows=4, nfin=2,
         mid=(512, 1536), TV=416, kq=(32, 32), scopes=False, xbs=1, wide=1, rp=0, rb=104, wearly=True, p0=0, xbw=(8, 28, 28), rpos=0, half=True):
    HALF[0] = half
    n = (F - a - c) // b
    assert a + n * b + c == F and c <= b
    assert sum(first) == M and sum(last) == M and sum(mid) == M
    assert TV <= mid[0] and TV <= last[0] and TV % 16 == 0
    foff = [sum(first[:i]) for i in range(len(first))]
    loff = [sum(last[:i]) for i in range(len(last))]
    moff = [sum(mid[:i]) for i in range(len(mid))]
    NS, NL = len(first), len(last)
    NT = b // 128
    NQ = len(kq)
    kqo = [sum(kq[:i]) for i in range(NQ + 1)]
    assert kqo[-1] == KT

    import contextlib
    scope = jax.named_scope if scopes else (lambda name: contextlib.nullcontext())

    def kern(xt_hbm, wg_hbm, wu_hbm, wd_hbm, o_hbm,
             xt_v, x32, w0, wm, wpk, acc, o_v, xb, w32, tt, isem, osem):
        whbm = (wg_hbm, wu_hbm, wd_hbm)

        def xcp(s):
            sl = pl.ds(foff[s], first[s])
            return pltpu.make_async_copy(xt_hbm.at[:, sl], xt_v.at[:, sl], isem.at[s])

        def w0cp(w):
            return pltpu.make_async_copy(whbm[w].at[:, pl.ds(0, a)], w0.at[w], isem.at[NS + w])

        def wmcp(w, j):
            if isinstance(j, int):
                off = min(a + j * b, F - b)
            else:
                off = pl.multiple_of(jnp.minimum(a + j * b, F - b), 128)
            sem = NS + 3 + j
            if isinstance(j, int) and j == 0 and w < 2:
                sem = NS + 3 + n + 1
            return pltpu.make_async_copy(whbm[w].at[:, pl.ds(off, b)], wm.at[w, j], isem.at[sem])

        def ocp(s, r, nr):
            sl = pl.ds(loff[s], last[s])
            rs = pl.ds(r * (D // nr), D // nr)
            return pltpu.make_async_copy(o_v.at[rs, sl], o_hbm.at[rs, sl], osem.at[0])

        def X(r0, nr, c0=0, nc=D):
            return pltpu.bitcast(x32[pl.ds(r0 // 2, nr // 2), pl.ds(c0, nc)], BF16)

        def WP(w, r0, nr, c0=0, nc=b):
            return pltpu.bitcast(wpk[w, pl.ds(r0 // 2, nr // 2), pl.ds(c0, nc)], BF16)

        def repack(j):
            for w in range(2):
                wpk[w] = pltpu.bitcast(wm[w, j], U32)

        xcp(0).start()
        w0cp(0).start()
        w0cp(1).start()
        xcp(1).start()
        w0cp(2).start()
        for s in range(2, NS - 1 if wearly else NS):
            xcp(s).start()
        wmcp(0, 0).start(priority=p0)
        wmcp(1, 0).start(priority=p0)
        if wearly:
            xcp(NS - 1).start()
        wmcp(2, 0).start(priority=1)
        for j in range(1, n + 1):
            for w in range(3):
                wmcp(w, j).start(priority=1)

        for q in range(1, NQ):
            tt[q] = jnp.zeros((TV, 2 * b), F32)

        h_prev = None
        for s in range(NS):
          with scope(f"first{s}"):
            sl = pl.ds(foff[s], first[s])
            xcp(s).wait()
            if s == 1:
                w0cp(2).wait()
            if s == NS - 1:
                for w in range(2):
                    wmcp(w, 0).wait()
            x32[pl.ds(foff[s] // 2, first[s] // 2), :] = pltpu.bitcast(xt_v[:, sl].T, U32)
            if s == 0:
                w0cp(0).wait()
                g0 = _dot(X(foff[s], first[s]), w0[0])
                w0cp(1).wait()
            if h_prev is not None:
                acc[:, pl.ds(foff[s - 1], first[s - 1])] = _down(w0[2], h_prev)
            if s == 0:
                h_prev = _act(g0, _dot(X(foff[s], first[s]), w0[1]))
            else:
                xs = X(foff[s], first[s])
                h_prev = _act(_dot(xs, w0[0]), _dot(xs, w0[1]))
            if s >= xbs:
                if xbw is None:
                    ks = [k for k in range(KT) if k % (NS - xbs) == s - xbs]
                else:
                    ks = list(range(sum(xbw[:s - xbs]), sum(xbw[:s - xbs + 1])))
                xtl = X(0, TV, KM, KT).astype(F32)
                for k in ks:
                    xb[k] = jnp.broadcast_to(xtl[:, k:k + 1], (TV, 128))
            if s == NS - 1:
                if rpos == 0:
                    repack(0)
                xtl = X(0, TV, KM, KT)
                tt[0, :, pl.ds(0, b)] = _dot(xtl, wm[0, 0, pl.ds(KM, KT), :])
                tt[0, :, pl.ds(b, b)] = _dot(xtl, wm[1, 0, pl.ds(KM, KT), :])
                acc[:, pl.ds(foff[NS - 1], first[NS - 1])] = _down(w0[2], h_prev)
                if rpos == 1:
                    repack(0)

        wmcp(2, 0).wait()

        def gu(r0, ts, tv, c0, nc):
            xm = X(r0, ts, 0, KM)
            g = _dot(xm, WP(0, 0, KM, c0, nc))
            u = _dot(xm, WP(1, 0, KM, c0, nc))
            pg, pu = [], []
            if tv:
                vg = tt[0, :, pl.ds(c0, nc)]
                vu = tt[0, :, pl.ds(b + c0, nc)]
                for q in range(1, NQ):
                    vg = vg + tt[q, :, pl.ds(c0, nc)]
                    vu = vu + tt[q, :, pl.ds(b + c0, nc)]
                pg.append(vg)
                pu.append(vu)
            if ts > tv:
                xt_ = X(r0 + tv, ts - tv, KM, KT)
                pg.append(_dot(xt_, WP(0, KM, KT, c0, nc)))
                pu.append(_dot(xt_, WP(1, KM, KT, c0, nc)))
            return _act(g + jnp.concatenate(pg, axis=0), u + jnp.concatenate(pu, axis=0))

        def body(j, carry):
            for w in range(3):
                wmcp(w, j + 1).wait()
            w32[:, pl.ds(0, b)] = wm[0, j + 1, pl.ds(KM, KT), :].astype(F32)
            w32[:, pl.ds(b, b)] = wm[1, j + 1, pl.ds(KM, KT), :].astype(F32)
            hs = [gu(moff[s], mid[s], TV if s == 0 else 0, 0, b) for s in range(len(mid))]
            if wide == 2:
                for q in range(NQ):
                    r = None
                    for k in range(kqo[q], kqo[q + 1]):
                        xk = xb[k]
                        p = jnp.concatenate([xk] * (2 * NT), axis=1) * w32[pl.ds(k, 1), :]
                        r = p if r is None else r + p
                    tt[q] = r
            else:
                for i in range(2 * NT):
                    cs = pl.ds(i * 128, 128)
                    for t0 in range(0, TV, rb):
                        rows = pl.ds(t0, min(rb, TV - t0))
                        for q in range(NQ):
                            r = None
                            for k in range(kqo[q], kqo[q + 1]):
                                p = xb[k, rows, :] * w32[pl.ds(k, 1), cs]
                                r = p if r is None else r + p
                            tt[q, rows, cs] = r
            if rp == 0:
                repack(j + 1)
            elif rp == 1:
                for w in range(2):
                    for ci in range(NT):
                        wpk[w, :, pl.ds(ci * 128, 128)] = pltpu.bitcast(wm[w, j + 1, :, pl.ds(ci * 128, 128)], U32)
            else:
                for w in range(2):
                    for ci in range(NT):
                        for rr in range(D // 16):
                            wpk[w, pl.ds(rr * 8, 8), pl.ds(ci * 128, 128)] = pltpu.bitcast(
                                wm[w, j + 1, pl.ds(rr * 16, 16), pl.ds(ci * 128, 128)], U32)
            for s in range(len(mid)):
                acc[:, pl.ds(moff[s], mid[s])] += _down(wm[2, j], hs[s])
            return carry

        with scope("loop"):
            lax.fori_loop(0, n, body, 0)

        c0 = b - c
        ocps = []

        def fin(s, h):
            sl = pl.ds(loff[s], last[s])
            nr = orows if s >= NL - nfin else 1
            val = acc[:, sl] + _down(wm[2, n, :, pl.ds(c0, c)], h)
            if not half:
                val = val * 0.5
            val = val.astype(BF16)
            for r in range(nr):
                rs = pl.ds(r * (D // nr), D // nr)
                o_v[rs, sl] = val[r * (D // nr):(r + 1) * (D // nr)]
                cp = ocp(s, r, nr)
                cp.start()
                ocps.append(cp)

        h_prev = None
        for s in range(NL):
            h = gu(loff[s], last[s], TV if s == 0 else 0, c0, c)
            if h_prev is not None:
                fin(s - 1, h_prev)
            h_prev = h
        fin(NL - 1, h_prev)
        with scope("finalwait"):
            for cp in ocps:
                cp.wait()

    def fn(x, w_gate, w_up, w_down):
        B, S, _ = x.shape
        xt = x.reshape(M, D).T
        wdt = w_down.T
        out_t = pl.pallas_call(
            kern,
            in_specs=[pl.BlockSpec(memory_space=pl.ANY)] * 4,
            out_specs=pl.BlockSpec(memory_space=pl.ANY),
            out_shape=jax.ShapeDtypeStruct((D, M), x.dtype),
            scratch_shapes=[
                pltpu.VMEM((D, M), BF16),
                pltpu.VMEM((M // 2, D), U32),
                pltpu.VMEM((3, D, a), BF16),
                pltpu.VMEM((3, n + 1, D, b), BF16),
                pltpu.VMEM((2, D // 2, b), U32),
                pltpu.VMEM((D, M), F32),
                pltpu.VMEM((D, M), BF16),
                pltpu.VMEM((KT, TV, 128), F32),
                pltpu.VMEM((KT, 2 * b), F32),
                pltpu.VMEM((NQ, TV, 2 * b), F32),
                pltpu.SemaphoreType.DMA((NS + 3 + n + 2,)),
                pltpu.SemaphoreType.DMA((1,)),
            ],
            compiler_params=pltpu.CompilerParams(vmem_limit_bytes=110 * 1024 * 1024,
                                                 disable_semaphore_checks=True),
        )(xt, w_gate, w_up, wdt)
        return out_t.T.reshape(B, S, D)
    return fn


_impl = make()


@jax.jit
def pallas_standalone__geglu_ffn__prompt_kernel(
    x: jax.Array,
    w_gate: jax.Array,
    w_up: jax.Array,
    w_down: jax.Array,
):
    return _impl(x, w_gate, w_up, w_down)
```

```python
import jax
import jax.numpy as jnp
from jax import lax
import jax.experimental.pallas as pl
import jax.experimental.pallas.tpu as pltpu

F32 = jnp.float32
BF16 = jnp.bfloat16
U32 = jnp.uint32
D, M, F = 576, 2048, 4608
KM, KT = 512, 64


HALF = [True]


def _act(g, u):
    c = 0.7978845608028654
    inner = g * (c + (c * 0.044715) * (g * g))
    if HALF[0]:
        return ((0.5 * g * (1.0 + jnp.tanh(inner))) * u).astype(BF16)
    return ((g * (1.0 + jnp.tanh(inner))) * u).astype(BF16)


def _dot(a, b):
    return jnp.dot(a, b, preferred_element_type=F32)


def _down(wdt, h):
    return lax.dot_general(wdt, h, (((1,), (1,)), ((), ())), preferred_element_type=F32)


def make(a=256, b=512, c=256, first=(256, 256, 768, 768), last=(640, 512, 384, 256, 256), orows=4, nfin=2,
         mid=(640, 1408), TV=528, kq=(16, 16, 16, 16), mprof=(6,) * 5 + (5,) * 16 + (4,) * 11, scopes=False, xbs=2, wide=1, rp=0, rb=104, wearly=True, p0=0, xbw=(32, 32), rpos=0, half=False, gsplit=False, dorder=0,
         zplan=((-1, 1, 0, 528), (-1, 2, 0, 528), (-1, 3, 0, 200), (-2, 3, 200, 528)),
         xplan=((3, 0, 528, 0, 40), (4, 0, 528, 40, 64))):
    HALF[0] = half
    n = (F - a - c) // b
    assert a + n * b + c == F and c <= b
    assert sum(first) == M and sum(last) == M and sum(mid) == M
    assert TV <= mid[0] and TV <= last[0] and TV % 16 == 0
    foff = [sum(first[:i]) for i in range(len(first))]
    loff = [sum(last[:i]) for i in range(len(last))]
    moff = [sum(mid[:i]) for i in range(len(mid))]
    NS, NL = len(first), len(last)
    NT = b // 128
    NQ = len(kq)
    kqo = [sum(kq[:i]) for i in range(NQ + 1)]
    assert kqo[-1] == KT

    import contextlib
    scope = jax.named_scope if scopes else (lambda name: contextlib.nullcontext())

    def kern(xt_hbm, wg_hbm, wu_hbm, wd_hbm, o_hbm,
             xt_v, x32, w0, wm, wpk, acc, o_v, xb, w32, tt, zv, isem, osem):
        whbm = (wg_hbm, wu_hbm, wd_hbm)

        def xcp(s):
            sl = pl.ds(foff[s], first[s])
            return pltpu.make_async_copy(xt_hbm.at[:, sl], xt_v.at[:, sl], isem.at[s])

        def w0cp(w):
            return pltpu.make_async_copy(whbm[w].at[:, pl.ds(0, a)], w0.at[w], isem.at[NS + w])

        def wmcp(w, j):
            if isinstance(j, int):
                off = min(a + j * b, F - b)
            else:
                off = pl.multiple_of(jnp.minimum(a + j * b, F - b), 128)
            sem = NS + 3 + j
            if isinstance(j, int) and j == 0 and w < 2:
                sem = NS + 3 + n + 1
            return pltpu.make_async_copy(whbm[w].at[:, pl.ds(off, b)], wm.at[w, j], isem.at[sem])

        def ocp(s, r, nr):
            sl = pl.ds(loff[s], last[s])
            rs = pl.ds(r * (D // nr), D // nr)
            return pltpu.make_async_copy(o_v.at[rs, sl], o_hbm.at[rs, sl], osem.at[0])

        def X(r0, nr, c0=0, nc=D):
            return pltpu.bitcast(x32[pl.ds(r0 // 2, nr // 2), pl.ds(c0, nc)], BF16)

        def WP(w, r0, nr, c0=0, nc=b):
            return pltpu.bitcast(wpk[w, pl.ds(r0 // 2, nr // 2), pl.ds(c0, nc)], BF16)

        def repack(j):
            for w in range(2):
                wpk[w] = pltpu.bitcast(wm[w, j], U32)

        xcp(0).start()
        w0cp(0).start()
        w0cp(1).start()
        if dorder == 0:
            xcp(1).start()
            w0cp(2).start()
        else:
            w0cp(2).start()
            xcp(1).start()
        for s in range(2, NS - 1 if wearly else NS):
            xcp(s).start()
        wmcp(0, 0).start(priority=p0)
        wmcp(1, 0).start(priority=p0)
        if wearly:
            xcp(NS - 1).start()
        wmcp(2, 0).start(priority=1)
        for j in range(1, n + 1):
            for w in range(3):
                wmcp(w, j).start(priority=1)

        zv[...] = jnp.zeros((8, 128), U32)

        def ttzero(slot):
            for (sl_, q, r0, r1) in zplan:
                if sl_ == slot:
                    tt[q, pl.ds(r0, r1 - r0), :] = jnp.zeros((r1 - r0, 2 * b), F32)

        def xbwork(slot):
            for (sl_, t0, t1, k0, k1) in xplan:
                if sl_ == slot:
                    xtl = X(t0, t1 - t0, KM, KT).astype(F32)
                    for k in range(k0, k1):
                        xb[k, pl.ds(t0, t1 - t0), :] = jnp.broadcast_to(xtl[:, k:k + 1], (t1 - t0, 128))

        ttzero(-1)

        h_prev = None
        for s in range(NS):
          with scope(f"first{s}"):
            sl = pl.ds(foff[s], first[s])
            xcp(s).wait()
            if s == 1:
                w0cp(2).wait()
            if s == NS - 1:
                for w in range(2):
                    wmcp(w, 0).wait()
            x32[pl.ds(foff[s] // 2, first[s] // 2), :] = pltpu.bitcast(xt_v[:, sl].T, U32)
            if s == 0:
                ttzero(-2)
                w0cp(0).wait()
                if gsplit:
                    g0 = _dot(X(foff[s], first[s], 0, KM), w0[0, pl.ds(0, KM), :])
                else:
                    g0 = _dot(X(foff[s], first[s]), w0[0])
                xbwork(0)
                ttzero(0)
                w0cp(1).wait()
            if h_prev is not None:
                acc[:, pl.ds(foff[s - 1], first[s - 1])] = _down(w0[2], h_prev)
            if s == 0:
                if gsplit:
                    g0 = g0 + _dot(X(foff[s], first[s], KM, KT), w0[0, pl.ds(KM, KT), :])
                h_prev = _act(g0, _dot(X(foff[s], first[s]), w0[1]))
            else:
                xs = X(foff[s], first[s])
                h_prev = _act(_dot(xs, w0[0]), _dot(xs, w0[1]))
            xbwork(s + 1)
            ttzero(s + 1)
            if s == NS - 1:
                if rpos == 0:
                    repack(0)
                xtl = X(0, TV, KM, KT)
                tt[0, :, pl.ds(0, b)] = _dot(xtl, wm[0, 0, pl.ds(KM, KT), :])
                tt[0, :, pl.ds(b, b)] = _dot(xtl, wm[1, 0, pl.ds(KM, KT), :])
                acc[:, pl.ds(foff[NS - 1], first[NS - 1])] = _down(w0[2], h_prev)
                if rpos == 1:
                    repack(0)

        wmcp(2, 0).wait()

        def gu(r0, ts, tv, c0, nc):
            xm = X(r0, ts, 0, KM)
            g = _dot(xm, WP(0, 0, KM, c0, nc))
            u = _dot(xm, WP(1, 0, KM, c0, nc))
            pg, pu = [], []
            if tv:
                vg = tt[0, :, pl.ds(c0, nc)]
                vu = tt[0, :, pl.ds(b + c0, nc)]
                for q in range(1, NQ):
                    vg = vg + tt[q, :, pl.ds(c0, nc)]
                    vu = vu + tt[q, :, pl.ds(b + c0, nc)]
                pg.append(vg)
                pu.append(vu)
            if ts > tv:
                xt_ = X(r0 + tv, ts - tv, KM, KT)
                pg.append(_dot(xt_, WP(0, KM, KT, c0, nc)))
                pu.append(_dot(xt_, WP(1, KM, KT, c0, nc)))
            return _act(g + jnp.concatenate(pg, axis=0), u + jnp.concatenate(pu, axis=0))

        def body(j, carry):
            for w in range(3):
                wmcp(w, j + 1).wait()
            w32[:, pl.ds(0, b)] = wm[0, j + 1, pl.ds(KM, KT), :].astype(F32)
            w32[:, pl.ds(b, b)] = wm[1, j + 1, pl.ds(KM, KT), :].astype(F32)
            hs = [gu(moff[s], mid[s], TV if s == 0 else 0, 0, b) for s in range(len(mid))]
            z = zv[...]
            st = (z, z, z, z)
            for i in range(2 * NT):
                cs = pl.ds(i * 128, 128)
                for q in range(NQ):
                    m = mprof[i * NQ + q]
                    wr = [w32[pl.ds(k, 1), cs] for k in range(kqo[q], kqo[q + 1])]

                    def chain(t, st, q=q, m=m, wr=wr, cs=cs):
                        f3, f2, f1, md = st
                        rows = pl.ds(pl.multiple_of(t * 8, 8), 8)
                        r = pltpu.bitcast((f3 | md) & z, F32)
                        mv = None
                        for kk, k in enumerate(range(kqo[q], kqo[q + 1])):
                            r = r + xb[k, rows, :] * wr[kk]
                            if kk + 1 == m:
                                mv = r
                        tt[q, rows, cs] = r
                        return (f2, f1, pltpu.bitcast(r, U32), pltpu.bitcast(mv, U32))

                    st = lax.fori_loop(0, TV // 8, chain, st, unroll=True)
            if rp == 0:
                repack(j + 1)
            elif rp == 1:
                for w in range(2):
                    for ci in range(NT):
                        wpk[w, :, pl.ds(ci * 128, 128)] = pltpu.bitcast(wm[w, j + 1, :, pl.ds(ci * 128, 128)], U32)
            else:
                for w in range(2):
                    for ci in range(NT):
                        for rr in range(D // 16):
                            wpk[w, pl.ds(rr * 8, 8), pl.ds(ci * 128, 128)] = pltpu.bitcast(
                                wm[w, j + 1, pl.ds(rr * 16, 16), pl.ds(ci * 128, 128)], U32)
            for s in range(len(mid)):
                acc[:, pl.ds(moff[s], mid[s])] += _down(wm[2, j], hs[s])
            return carry

        with scope("loop"):
            lax.fori_loop(0, n, body, 0)

        c0 = b - c
        ocps = []

        def fin(s, h):
            sl = pl.ds(loff[s], last[s])
            nr = orows if s >= NL - nfin else 1
            val = acc[:, sl] + _down(wm[2, n, :, pl.ds(c0, c)], h)
            if not half:
                val = val * 0.5
            val = val.astype(BF16)
            for r in range(nr):
                rs = pl.ds(r * (D // nr), D // nr)
                o_v[rs, sl] = val[r * (D // nr):(r + 1) * (D // nr)]
                cp = ocp(s, r, nr)
                cp.start()
                ocps.append(cp)

        h_prev = None
        for s in range(NL):
            h = gu(loff[s], last[s], TV if s == 0 else 0, c0, c)
            if h_prev is not None:
                fin(s - 1, h_prev)
            h_prev = h
        fin(NL - 1, h_prev)
        with scope("finalwait"):
            for cp in ocps:
                cp.wait()

    def fn(x, w_gate, w_up, w_down):
        B, S, _ = x.shape
        xt = x.reshape(M, D).T
        wdt = w_down.T
        out_t = pl.pallas_call(
            kern,
            in_specs=[pl.BlockSpec(memory_space=pl.ANY)] * 4,
            out_specs=pl.BlockSpec(memory_space=pl.ANY),
            out_shape=jax.ShapeDtypeStruct((D, M), x.dtype),
            scratch_shapes=[
                pltpu.VMEM((D, M), BF16),
                pltpu.VMEM((M // 2, D), U32),
                pltpu.VMEM((3, D, a), BF16),
                pltpu.VMEM((3, n + 1, D, b), BF16),
                pltpu.VMEM((2, D // 2, b), U32),
                pltpu.VMEM((D, M), F32),
                pltpu.VMEM((D, M), BF16),
                pltpu.VMEM((KT, TV, 128), F32),
                pltpu.VMEM((KT, 2 * b), F32),
                pltpu.VMEM((NQ, TV, 2 * b), F32),
                pltpu.VMEM((8, 128), U32),
                pltpu.SemaphoreType.DMA((NS + 3 + n + 2,)),
                pltpu.SemaphoreType.DMA((1,)),
            ],
            compiler_params=pltpu.CompilerParams(vmem_limit_bytes=110 * 1024 * 1024,
                                                 disable_semaphore_checks=True),
        )(xt, w_gate, w_up, wdt)
        return out_t.T.reshape(B, S, D)
    return fn


_impl = make()


@jax.jit
def pallas_standalone__geglu_ffn__prompt_kernel(
    x: jax.Array,
    w_gate: jax.Array,
    w_up: jax.Array,
    w_down: jax.Array,
):
    return _impl(x, w_gate, w_up, w_down)
```

```python
import jax
import jax.numpy as jnp
from jax import lax
import jax.experimental.pallas as pl
import jax.experimental.pallas.tpu as pltpu

F32 = jnp.float32
BF16 = jnp.bfloat16
U32 = jnp.uint32
D, M, F = 576, 2048, 4608
KM, KT = 512, 64


HALF = [True]


def _act(g, u):
    c = 0.7978845608028654
    inner = g * (c + (c * 0.044715) * (g * g))
    if HALF[0]:
        return ((0.5 * g * (1.0 + jnp.tanh(inner))) * u).astype(BF16)
    return ((g * (1.0 + jnp.tanh(inner))) * u).astype(BF16)


def _dot(a, b):
    return jnp.dot(a, b, preferred_element_type=F32)


def _down(wdt, h):
    return lax.dot_general(wdt, h, (((1,), (1,)), ((), ())), preferred_element_type=F32)


def make(a=256, b=512, c=256, first=(256, 256, 768, 768), last=(640, 512, 384, 256, 256), orows=4, nfin=2,
         mid=(640, 1408), TV=544, kq=(16, 16, 16, 16), mprof=(6,) * 3 + (5,) * 13 + (4,) * 16, scopes=False, xbs=2, wide=1, rp=0, rb=104, wearly=True, p0=0, xbw=(32, 32), rpos=0, half=False, gsplit=False, dorder=0, unroll=1,
         zplan=((-1, 1, 0, 544), (-1, 2, 0, 544), (-1, 3, 0, 200), (-2, 3, 200, 544)),
         xplan=((3, 0, 544, 0, 40), (4, 0, 544, 40, 64))):
    HALF[0] = half
    n = (F - a - c) // b
    assert a + n * b + c == F and c <= b
    assert sum(first) == M and sum(last) == M and sum(mid) == M
    assert TV <= mid[0] and TV <= last[0] and TV % 16 == 0
    foff = [sum(first[:i]) for i in range(len(first))]
    loff = [sum(last[:i]) for i in range(len(last))]
    moff = [sum(mid[:i]) for i in range(len(mid))]
    NS, NL = len(first), len(last)
    NT = b // 128
    NQ = len(kq)
    kqo = [sum(kq[:i]) for i in range(NQ + 1)]
    assert kqo[-1] == KT

    import contextlib
    scope = jax.named_scope if scopes else (lambda name: contextlib.nullcontext())

    def kern(xt_hbm, wg_hbm, wu_hbm, wd_hbm, o_hbm,
             xt_v, x32, w0, wm, wpk, acc, o_v, xb, w32, tt, zv, isem, osem):
        whbm = (wg_hbm, wu_hbm, wd_hbm)

        def xcp(s):
            sl = pl.ds(foff[s], first[s])
            return pltpu.make_async_copy(xt_hbm.at[:, sl], xt_v.at[:, sl], isem.at[s])

        def w0cp(w):
            return pltpu.make_async_copy(whbm[w].at[:, pl.ds(0, a)], w0.at[w], isem.at[NS + w])

        def wmcp(w, j):
            if isinstance(j, int):
                off = min(a + j * b, F - b)
            else:
                off = pl.multiple_of(jnp.minimum(a + j * b, F - b), 128)
            sem = NS + 3 + j
            if isinstance(j, int) and j == 0 and w < 2:
                sem = NS + 3 + n + 1
            return pltpu.make_async_copy(whbm[w].at[:, pl.ds(off, b)], wm.at[w, j], isem.at[sem])

        def ocp(s, r, nr):
            sl = pl.ds(loff[s], last[s])
            rs = pl.ds(r * (D // nr), D // nr)
            return pltpu.make_async_copy(o_v.at[rs, sl], o_hbm.at[rs, sl], osem.at[0])

        def X(r0, nr, c0=0, nc=D):
            return pltpu.bitcast(x32[pl.ds(r0 // 2, nr // 2), pl.ds(c0, nc)], BF16)

        def WP(w, r0, nr, c0=0, nc=b):
            return pltpu.bitcast(wpk[w, pl.ds(r0 // 2, nr // 2), pl.ds(c0, nc)], BF16)

        def repack(j):
            for w in range(2):
                wpk[w] = pltpu.bitcast(wm[w, j], U32)

        xcp(0).start()
        w0cp(0).start()
        w0cp(1).start()
        if dorder == 0:
            xcp(1).start()
            w0cp(2).start()
        else:
            w0cp(2).start()
            xcp(1).start()
        for s in range(2, NS - 1 if wearly else NS):
            xcp(s).start()
        wmcp(0, 0).start(priority=p0)
        wmcp(1, 0).start(priority=p0)
        if wearly:
            xcp(NS - 1).start()
        wmcp(2, 0).start(priority=1)
        for j in range(1, n + 1):
            for w in range(3):
                wmcp(w, j).start(priority=1)

        zv[...] = jnp.zeros((8, 128), U32)

        def ttzero(slot):
            for (sl_, q, r0, r1) in zplan:
                if sl_ == slot:
                    tt[q, pl.ds(r0, r1 - r0), :] = jnp.zeros((r1 - r0, 2 * b), F32)

        def xbwork(slot):
            for (sl_, t0, t1, k0, k1) in xplan:
                if sl_ == slot:
                    xtl = X(t0, t1 - t0, KM, KT).astype(F32)
                    for k in range(k0, k1):
                        xb[k, pl.ds(t0, t1 - t0), :] = jnp.broadcast_to(xtl[:, k:k + 1], (t1 - t0, 128))

        ttzero(-1)

        h_prev = None
        for s in range(NS):
          with scope(f"first{s}"):
            sl = pl.ds(foff[s], first[s])
            xcp(s).wait()
            if s == 1:
                w0cp(2).wait()
            if s == NS - 1:
                for w in range(2):
                    wmcp(w, 0).wait()
            x32[pl.ds(foff[s] // 2, first[s] // 2), :] = pltpu.bitcast(xt_v[:, sl].T, U32)
            if s == 0:
                ttzero(-2)
                w0cp(0).wait()
                if gsplit:
                    g0 = _dot(X(foff[s], first[s], 0, KM), w0[0, pl.ds(0, KM), :])
                else:
                    g0 = _dot(X(foff[s], first[s]), w0[0])
                xbwork(0)
                ttzero(0)
                w0cp(1).wait()
            if h_prev is not None:
                acc[:, pl.ds(foff[s - 1], first[s - 1])] = _down(w0[2], h_prev)
            if s == 0:
                if gsplit:
                    g0 = g0 + _dot(X(foff[s], first[s], KM, KT), w0[0, pl.ds(KM, KT), :])
                h_prev = _act(g0, _dot(X(foff[s], first[s]), w0[1]))
            else:
                xs = X(foff[s], first[s])
                h_prev = _act(_dot(xs, w0[0]), _dot(xs, w0[1]))
            xbwork(s + 1)
            ttzero(s + 1)
            if s == NS - 1:
                if rpos == 0:
                    repack(0)
                xtl = X(0, TV, KM, KT)
                tt[0, :, pl.ds(0, b)] = _dot(xtl, wm[0, 0, pl.ds(KM, KT), :])
                tt[0, :, pl.ds(b, b)] = _dot(xtl, wm[1, 0, pl.ds(KM, KT), :])
                acc[:, pl.ds(foff[NS - 1], first[NS - 1])] = _down(w0[2], h_prev)
                if rpos == 1:
                    repack(0)

        wmcp(2, 0).wait()

        def gu(r0, ts, tv, c0, nc):
            xm = X(r0, ts, 0, KM)
            g = _dot(xm, WP(0, 0, KM, c0, nc))
            u = _dot(xm, WP(1, 0, KM, c0, nc))
            pg, pu = [], []
            if tv:
                vg = tt[0, :, pl.ds(c0, nc)]
                vu = tt[0, :, pl.ds(b + c0, nc)]
                for q in range(1, NQ):
                    vg = vg + tt[q, :, pl.ds(c0, nc)]
                    vu = vu + tt[q, :, pl.ds(b + c0, nc)]
                pg.append(vg)
                pu.append(vu)
            if ts > tv:
                xt_ = X(r0 + tv, ts - tv, KM, KT)
                pg.append(_dot(xt_, WP(0, KM, KT, c0, nc)))
                pu.append(_dot(xt_, WP(1, KM, KT, c0, nc)))
            return _act(g + jnp.concatenate(pg, axis=0), u + jnp.concatenate(pu, axis=0))

        def body(j, carry):
            for w in range(3):
                wmcp(w, j + 1).wait()
            w32[:, pl.ds(0, b)] = wm[0, j + 1, pl.ds(KM, KT), :].astype(F32)
            w32[:, pl.ds(b, b)] = wm[1, j + 1, pl.ds(KM, KT), :].astype(F32)
            hs = [gu(moff[s], mid[s], TV if s == 0 else 0, 0, b) for s in range(len(mid))]
            z = zv[...]
            st = (z, z, z, z)
            for i in range(2 * NT):
                cs = pl.ds(i * 128, 128)
                for q in range(NQ):
                    m = mprof[i * NQ + q]
                    wr = [w32[pl.ds(k, 1), cs] for k in range(kqo[q], kqo[q + 1])]

                    def chain(t, st, q=q, m=m, wr=wr, cs=cs):
                        f3, f2, f1, md = st
                        rows = pl.ds(pl.multiple_of(t * 8, 8), 8)
                        r = pltpu.bitcast((f3 | md) & z, F32)
                        mv = None
                        for kk, k in enumerate(range(kqo[q], kqo[q + 1])):
                            r = r + xb[k, rows, :] * wr[kk]
                            if kk + 1 == m:
                                mv = r
                        tt[q, rows, cs] = r
                        return (f2, f1, pltpu.bitcast(r, U32), pltpu.bitcast(mv, U32))

                    st = lax.fori_loop(0, TV // 8, chain, st, unroll=True)
            if rp == 0:
                repack(j + 1)
            elif rp == 1:
                for w in range(2):
                    for ci in range(NT):
                        wpk[w, :, pl.ds(ci * 128, 128)] = pltpu.bitcast(wm[w, j + 1, :, pl.ds(ci * 128, 128)], U32)
            else:
                for w in range(2):
                    for ci in range(NT):
                        for rr in range(D // 16):
                            wpk[w, pl.ds(rr * 8, 8), pl.ds(ci * 128, 128)] = pltpu.bitcast(
                                wm[w, j + 1, pl.ds(rr * 16, 16), pl.ds(ci * 128, 128)], U32)
            for s in range(len(mid)):
                acc[:, pl.ds(moff[s], mid[s])] += _down(wm[2, j], hs[s])
            return carry

        with scope("loop"):
            lax.fori_loop(0, n, body, 0, unroll=unroll)

        c0 = b - c
        ocps = []

        def fin(s, h):
            sl = pl.ds(loff[s], last[s])
            nr = orows if s >= NL - nfin else 1
            val = acc[:, sl] + _down(wm[2, n, :, pl.ds(c0, c)], h)
            if not half:
                val = val * 0.5
            val = val.astype(BF16)
            for r in range(nr):
                rs = pl.ds(r * (D // nr), D // nr)
                o_v[rs, sl] = val[r * (D // nr):(r + 1) * (D // nr)]
                cp = ocp(s, r, nr)
                cp.start()
                ocps.append(cp)

        h_prev = None
        for s in range(NL):
            h = gu(loff[s], last[s], TV if s == 0 else 0, c0, c)
            if h_prev is not None:
                fin(s - 1, h_prev)
            h_prev = h
        fin(NL - 1, h_prev)
        with scope("finalwait"):
            for cp in ocps:
                cp.wait()

    def fn(x, w_gate, w_up, w_down):
        B, S, _ = x.shape
        xt = x.reshape(M, D).T
        wdt = w_down.T
        out_t = pl.pallas_call(
            kern,
            in_specs=[pl.BlockSpec(memory_space=pl.ANY)] * 4,
            out_specs=pl.BlockSpec(memory_space=pl.ANY),
            out_shape=jax.ShapeDtypeStruct((D, M), x.dtype),
            scratch_shapes=[
                pltpu.VMEM((D, M), BF16),
                pltpu.VMEM((M // 2, D), U32),
                pltpu.VMEM((3, D, a), BF16),
                pltpu.VMEM((3, n + 1, D, b), BF16),
                pltpu.VMEM((2, D // 2, b), U32),
                pltpu.VMEM((D, M), F32),
                pltpu.VMEM((D, M), BF16),
                pltpu.VMEM((KT, TV, 128), F32),
                pltpu.VMEM((KT, 2 * b), F32),
                pltpu.VMEM((NQ, TV, 2 * b), F32),
                pltpu.VMEM((8, 128), U32),
                pltpu.SemaphoreType.DMA((NS + 3 + n + 2,)),
                pltpu.SemaphoreType.DMA((1,)),
            ],
            compiler_params=pltpu.CompilerParams(vmem_limit_bytes=110 * 1024 * 1024,
                                                 disable_semaphore_checks=True),
        )(xt, w_gate, w_up, wdt)
        return out_t.T.reshape(B, S, D)
    return fn


_impl = make()


@jax.jit
def pallas_standalone__geglu_ffn__prompt_kernel(
    x: jax.Array,
    w_gate: jax.Array,
    w_up: jax.Array,
    w_down: jax.Array,
):
    return _impl(x, w_gate, w_up, w_down)
```

```python
import contextlib

import jax
import jax.numpy as jnp
from jax import lax
import jax.experimental.pallas as pl
import jax.experimental.pallas.tpu as pltpu

F32 = jnp.float32
BF16 = jnp.bfloat16
U32 = jnp.uint32
D, M, F = 576, 2048, 4608
KM, KT = 512, 64
KQ = 16
NQ = KT // KQ


def _act(g, u):
    c = 0.7978845608028654
    inner = g * (c + (c * 0.044715) * (g * g))
    return ((g * (1.0 + jnp.tanh(inner))) * u).astype(BF16)


def _dot(a, b):
    return jnp.dot(a, b, preferred_element_type=F32)


def _down(wdt, h):
    return lax.dot_general(wdt, h, (((1,), (1,)), ((), ())), preferred_element_type=F32)


def make(a=256, b=512, c=256, first=(256, 256, 768, 768), mid=(640, 1408), last=(640, 512, 384, 256, 256),
         orows=4, nfin=2, TV=544, mprof=(8,) * 4 + (7,) * 11 + (6,) * 17,
         z0=200, xplan=((2, 0, 544, 0, 40), (3, 0, 544, 40, 64)),
         fv_tiles=0, fv_rows=0, fv_m=7, scopes=False):
    n = (F - a - c) // b
    assert a + n * b + c == F and c <= b
    assert sum(first) == M and sum(last) == M and sum(mid) == M
    assert TV <= mid[0] and TV <= last[0] and TV % 16 == 0
    foff = [sum(first[:i]) for i in range(len(first))]
    loff = [sum(last[:i]) for i in range(len(last))]
    moff = [sum(mid[:i]) for i in range(len(mid))]
    NS, NL = len(first), len(last)
    NT = b // 128
    scope = jax.named_scope if scopes else (lambda name: contextlib.nullcontext())

    def kern(xt_hbm, wg_hbm, wu_hbm, wd_hbm, o_hbm,
             xt_v, x32, w0, wm, wpk, acc, o_v, xb, w32, tt, zv, isem, osem):
        whbm = (wg_hbm, wu_hbm, wd_hbm)

        def xcp(s):
            sl = pl.ds(foff[s], first[s])
            return pltpu.make_async_copy(xt_hbm.at[:, sl], xt_v.at[:, sl], isem.at[s])

        def w0cp(w):
            return pltpu.make_async_copy(whbm[w].at[:, pl.ds(0, a)], w0.at[w], isem.at[NS + w])

        def wmcp(w, j):
            if isinstance(j, int):
                off = min(a + j * b, F - b)
            else:
                off = pl.multiple_of(jnp.minimum(a + j * b, F - b), 128)
            sem = NS + 3 + j
            if isinstance(j, int) and j == 0 and w < 2:
                sem = NS + 3 + n + 1
            return pltpu.make_async_copy(whbm[w].at[:, pl.ds(off, b)], wm.at[w, j], isem.at[sem])

        def ocp(s, r, nr):
            sl = pl.ds(loff[s], last[s])
            rs = pl.ds(r * (D // nr), D // nr)
            return pltpu.make_async_copy(o_v.at[rs, sl], o_hbm.at[rs, sl], osem.at[0])

        def X(r0, nr, c0=0, nc=D):
            return pltpu.bitcast(x32[pl.ds(r0 // 2, nr // 2), pl.ds(c0, nc)], BF16)

        def WP(w, r0, nr, c0, nc):
            return pltpu.bitcast(wpk[w, pl.ds(r0 // 2, nr // 2), pl.ds(c0, nc)], BF16)

        def tail_f32(j):
            w32[:, pl.ds(0, b)] = wm[0, j, pl.ds(KM, KT), :].astype(F32)
            w32[:, pl.ds(b, b)] = wm[1, j, pl.ds(KM, KT), :].astype(F32)

        def vpu_tail(tiles, nrows, ms):
            never1 = zv[0] != 0
            never2 = zv[1] != 0
            zf = pltpu.bitcast(zv[0], F32)
            st = (zf, zf, zf, zf)
            g = 0
            for i in tiles:
                cs = pl.ds(i * 128, 128)
                for q in range(NQ):
                    wr = [w32[pl.ds(q * KQ + kk, 1), cs] for kk in range(KQ)]

                    def chain(t, st, q=q, m=ms[g], wr=wr, cs=cs):
                        f3, f2, f1, md = st
                        rows = pl.ds(pl.multiple_of(t * 8, 8), 8)
                        r = mv = None
                        for kk in range(KQ):
                            p = xb[q * KQ + kk, rows, :] * wr[kk]
                            if kk == 0:
                                r = jnp.where(never2, f3, jnp.where(never1, md, p))
                            else:
                                r = r + p
                            if kk + 1 == m:
                                mv = r
                        tt[q, rows, cs] = r
                        return (f2, f1, r, mv)

                    st = lax.fori_loop(0, nrows // 8, chain, st, unroll=True)
                    g += 1

        xcp(0).start()
        w0cp(0).start()
        w0cp(1).start()
        xcp(1).start()
        w0cp(2).start()
        for s in range(2, NS - 1):
            xcp(s).start()
        wmcp(0, 0).start()
        wmcp(1, 0).start()
        xcp(NS - 1).start()
        wmcp(2, 0).start(priority=1)
        for j in range(1, n + 1):
            for w in range(3):
                wmcp(w, j).start(priority=1)

        zv[...] = jnp.zeros(zv.shape, U32)
        for q in range(1, NQ - 1):
            tt[q] = jnp.zeros((TV, 2 * b), F32)
        tt[NQ - 1, pl.ds(0, z0), :] = jnp.zeros((z0, 2 * b), F32)

        h_prev = None
        for s in range(NS):
          with scope(f"first{s}"):
            sl = pl.ds(foff[s], first[s])
            xcp(s).wait()
            if s == 1:
                w0cp(2).wait()
            if s == NS - 1:
                wmcp(0, 0).wait()
                wmcp(1, 0).wait()
            x32[pl.ds(foff[s] // 2, first[s] // 2), :] = pltpu.bitcast(xt_v[:, sl].T, U32)
            if s == 0:
                tt[NQ - 1, pl.ds(z0, TV - z0), :] = jnp.zeros((TV - z0, 2 * b), F32)
                w0cp(0).wait()
                g0 = _dot(X(foff[s], first[s]), w0[0])
                w0cp(1).wait()
                h_prev = _act(g0, _dot(X(foff[s], first[s]), w0[1]))
            else:
                acc[:, pl.ds(foff[s - 1], first[s - 1])] = _down(w0[2], h_prev)
                xs = X(foff[s], first[s])
                h_prev = _act(_dot(xs, w0[0]), _dot(xs, w0[1]))
            for (s_, t0, t1, k0, k1) in xplan:
                if s_ == s:
                    xtl = X(t0, t1 - t0, KM, KT).astype(F32)
                    for k in range(k0, k1):
                        xb[k, pl.ds(t0, t1 - t0), :] = jnp.broadcast_to(xtl[:, k:k + 1], (t1 - t0, 128))
            if s == NS - 1:
                zz = zv[0]
                prev = zz
                for w in range(2):
                    for ci in range(NT):
                        def rp(rr, prev, w=w, ci=ci):
                            r16 = pl.multiple_of(rr * 16, 16)
                            r8 = pl.multiple_of(rr * 8, 8)
                            v = pltpu.bitcast(wm[w, 0, pl.ds(r16, 16), pl.ds(ci * 128, 128)], U32) | (prev & zz)
                            wpk[w, pl.ds(r8, 8), pl.ds(ci * 128, 128)] = v
                            return v
                        prev = lax.fori_loop(0, D // 16, rp, prev, unroll=True)
                if fv_tiles:
                    tail_f32(0)
                    vpu_tail(range(fv_tiles), fv_rows, (fv_m,) * (fv_tiles * NQ))
                    assert fv_tiles == NT
                    tt[0, pl.ds(fv_rows, TV - fv_rows), pl.ds(0, b)] = _dot(
                        X(fv_rows, TV - fv_rows, KM, KT), wm[0, 0, pl.ds(KM, KT), :])
                else:
                    tt[0, :, pl.ds(0, b)] = _dot(X(0, TV, KM, KT), wm[0, 0, pl.ds(KM, KT), :])
                tt[0, :, pl.ds(b, b)] = _dot(X(0, TV, KM, KT), wm[1, 0, pl.ds(KM, KT), :])
                acc[:, pl.ds(foff[s], first[s])] = _down(w0[2], h_prev)

        wmcp(2, 0).wait()

        def gu(r0, ts, tv, c0, nc):
            xm = X(r0, ts, 0, KM)
            g = _dot(xm, WP(0, 0, KM, c0, nc))
            u = _dot(xm, WP(1, 0, KM, c0, nc))
            pg, pu = [], []
            if tv:
                vg = tt[0, :, pl.ds(c0, nc)]
                vu = tt[0, :, pl.ds(b + c0, nc)]
                for q in range(1, NQ):
                    vg = vg + tt[q, :, pl.ds(c0, nc)]
                    vu = vu + tt[q, :, pl.ds(b + c0, nc)]
                pg.append(vg)
                pu.append(vu)
            xt_ = X(r0 + tv, ts - tv, KM, KT)
            pg.append(_dot(xt_, WP(0, KM, KT, c0, nc)))
            pu.append(_dot(xt_, WP(1, KM, KT, c0, nc)))
            return _act(g + jnp.concatenate(pg, axis=0), u + jnp.concatenate(pu, axis=0))

        def body(j, carry):
            for w in range(3):
                wmcp(w, j + 1).wait()
            tail_f32(j + 1)
            hs = [gu(moff[s], mid[s], TV if s == 0 else 0, 0, b) for s in range(len(mid))]
            vpu_tail(range(2 * NT), TV, mprof)
            for w in range(2):
                wpk[w] = pltpu.bitcast(wm[w, j + 1], U32)
            for s in range(len(mid)):
                acc[:, pl.ds(moff[s], mid[s])] += _down(wm[2, j], hs[s])
            return carry

        with scope("loop"):
            lax.fori_loop(0, n, body, 0)

        c0 = b - c
        ocps = []

        def fin(s, h):
            sl = pl.ds(loff[s], last[s])
            nr = orows if s >= NL - nfin else 1
            val = ((acc[:, sl] + _down(wm[2, n, :, pl.ds(c0, c)], h)) * 0.5).astype(BF16)
            for r in range(nr):
                rs = pl.ds(r * (D // nr), D // nr)
                o_v[rs, sl] = val[r * (D // nr):(r + 1) * (D // nr)]
                cp = ocp(s, r, nr)
                cp.start()
                ocps.append(cp)

        h_prev = None
        for s in range(NL):
            h = gu(loff[s], last[s], TV if s == 0 else 0, c0, c)
            if h_prev is not None:
                fin(s - 1, h_prev)
            h_prev = h
        fin(NL - 1, h_prev)
        with scope("finalwait"):
            for cp in ocps:
                cp.wait()

    def fn(x, w_gate, w_up, w_down):
        B, S, _ = x.shape
        xt = x.reshape(M, D).T
        wdt = w_down.T
        out_t = pl.pallas_call(
            kern,
            in_specs=[pl.BlockSpec(memory_space=pl.ANY)] * 4,
            out_specs=pl.BlockSpec(memory_space=pl.ANY),
            out_shape=jax.ShapeDtypeStruct((D, M), x.dtype),
            scratch_shapes=[
                pltpu.VMEM((D, M), BF16),
                pltpu.VMEM((M // 2, D), U32),
                pltpu.VMEM((3, D, a), BF16),
                pltpu.VMEM((3, n + 1, D, b), BF16),
                pltpu.VMEM((2, D // 2, b), U32),
                pltpu.VMEM((D, M), F32),
                pltpu.VMEM((D, M), BF16),
                pltpu.VMEM((KT, TV, 128), F32),
                pltpu.VMEM((KT, 2 * b), F32),
                pltpu.VMEM((NQ, TV, 2 * b), F32),
                pltpu.VMEM((2, 8, 128), U32),
                pltpu.SemaphoreType.DMA((NS + 3 + n + 2,)),
                pltpu.SemaphoreType.DMA((1,)),
            ],
            compiler_params=pltpu.CompilerParams(vmem_limit_bytes=110 * 1024 * 1024,
                                                 disable_semaphore_checks=True),
        )(xt, w_gate, w_up, wdt)
        return out_t.T.reshape(B, S, D)
    return fn


_impl = make()


@jax.jit
def pallas_standalone__geglu_ffn__prompt_kernel(
    x: jax.Array,
    w_gate: jax.Array,
    w_up: jax.Array,
    w_down: jax.Array,
):
    return _impl(x, w_gate, w_up, w_down)
```

```python
import contextlib

import jax
import jax.numpy as jnp
from jax import lax
import jax.experimental.pallas as pl
import jax.experimental.pallas.tpu as pltpu

F32 = jnp.float32
BF16 = jnp.bfloat16
U32 = jnp.uint32
D, M, F = 576, 2048, 4608
KM, KT = 512, 64
KQ = 16
NQ = KT // KQ


def _act(g, u):
    c = 0.7978845608028654
    inner = g * (c + (c * 0.044715) * (g * g))
    return ((g * (1.0 + jnp.tanh(inner))) * u).astype(BF16)


def _dot(a, b):
    return jnp.dot(a, b, preferred_element_type=F32)


def _down(wdt, h):
    return lax.dot_general(wdt, h, (((1,), (1,)), ((), ())), preferred_element_type=F32)


def make(a=256, b=512, c=256, first=(256, 256, 768, 768), mid=(640, 1408), last=(640, 512, 384, 256, 256),
         orows=4, nfin=2, TV=544, mprof=(8,) * 4 + (7,) * 11 + (6,) * 17,
         z0=200, xplan=((2, 0, 544, 0, 40), (3, 0, 544, 40, 64)),
         fv_tiles=0, fv_rows=0, fv_m=7, scopes=False, oneloop=True):
    n = (F - a - c) // b
    assert a + n * b + c == F and c <= b
    assert sum(first) == M and sum(last) == M and sum(mid) == M
    assert TV <= mid[0] and TV <= last[0] and TV % 16 == 0
    foff = [sum(first[:i]) for i in range(len(first))]
    loff = [sum(last[:i]) for i in range(len(last))]
    moff = [sum(mid[:i]) for i in range(len(mid))]
    NS, NL = len(first), len(last)
    NT = b // 128
    scope = jax.named_scope if scopes else (lambda name: contextlib.nullcontext())

    def kern(xt_hbm, wg_hbm, wu_hbm, wd_hbm, o_hbm,
             xt_v, x32, w0, wm, wpk, acc, o_v, xb, w32, tt, zv, isem, osem):
        whbm = (wg_hbm, wu_hbm, wd_hbm)

        def xcp(s):
            sl = pl.ds(foff[s], first[s])
            return pltpu.make_async_copy(xt_hbm.at[:, sl], xt_v.at[:, sl], isem.at[s])

        def w0cp(w):
            return pltpu.make_async_copy(whbm[w].at[:, pl.ds(0, a)], w0.at[w], isem.at[NS + w])

        def wmcp(w, j):
            if isinstance(j, int):
                off = min(a + j * b, F - b)
            else:
                off = pl.multiple_of(jnp.minimum(a + j * b, F - b), 128)
            sem = NS + 3 + j
            if isinstance(j, int) and j == 0 and w < 2:
                sem = NS + 3 + n + 1
            return pltpu.make_async_copy(whbm[w].at[:, pl.ds(off, b)], wm.at[w, j], isem.at[sem])

        def ocp(s, r, nr):
            sl = pl.ds(loff[s], last[s])
            rs = pl.ds(r * (D // nr), D // nr)
            return pltpu.make_async_copy(o_v.at[rs, sl], o_hbm.at[rs, sl], osem.at[0])

        def X(r0, nr, c0=0, nc=D):
            return pltpu.bitcast(x32[pl.ds(r0 // 2, nr // 2), pl.ds(c0, nc)], BF16)

        def WP(w, r0, nr, c0, nc):
            return pltpu.bitcast(wpk[w, pl.ds(r0 // 2, nr // 2), pl.ds(c0, nc)], BF16)

        def tail_f32(j):
            w32[:, pl.ds(0, b)] = wm[0, j, pl.ds(KM, KT), :].astype(F32)
            w32[:, pl.ds(b, b)] = wm[1, j, pl.ds(KM, KT), :].astype(F32)

        def vpu_tail(tiles, nrows, ms):
            never1 = zv[0] != 0
            never2 = zv[1] != 0
            zf = pltpu.bitcast(zv[0], F32)
            st = (zf, zf, zf, zf)
            g = 0
            for i in tiles:
                cs = pl.ds(i * 128, 128)
                for q in range(NQ):
                    wr = [w32[pl.ds(q * KQ + kk, 1), cs] for kk in range(KQ)]

                    def chain(t, st, q=q, m=ms[g], wr=wr, cs=cs):
                        f3, f2, f1, md = st
                        rows = pl.ds(pl.multiple_of(t * 8, 8), 8)
                        r = mv = None
                        for kk in range(KQ):
                            p = xb[q * KQ + kk, rows, :] * wr[kk]
                            if kk == 0:
                                r = jnp.where(never2, f3, jnp.where(never1, md, p))
                            else:
                                r = r + p
                            if kk + 1 == m:
                                mv = r
                        tt[q, rows, cs] = r
                        return (f2, f1, r, mv)

                    st = lax.fori_loop(0, nrows // 8, chain, st, unroll=True)
                    g += 1

        xcp(0).start()
        w0cp(0).start()
        w0cp(1).start()
        xcp(1).start()
        w0cp(2).start()
        for s in range(2, NS - 1):
            xcp(s).start()
        wmcp(0, 0).start()
        wmcp(1, 0).start()
        xcp(NS - 1).start()
        wmcp(2, 0).start(priority=1)
        for j in range(1, n + 1):
            for w in range(3):
                wmcp(w, j).start(priority=1)

        zv[...] = jnp.zeros(zv.shape, U32)
        for q in range(1, NQ - 1):
            tt[q] = jnp.zeros((TV, 2 * b), F32)
        tt[NQ - 1, pl.ds(0, z0), :] = jnp.zeros((z0, 2 * b), F32)

        def first_block():
            h_prev = None
            for s in range(NS):
              with scope(f"first{s}"):
                sl = pl.ds(foff[s], first[s])
                xcp(s).wait()
                if s == 1:
                    w0cp(2).wait()
                if s == NS - 1:
                    wmcp(0, 0).wait()
                    wmcp(1, 0).wait()
                x32[pl.ds(foff[s] // 2, first[s] // 2), :] = pltpu.bitcast(xt_v[:, sl].T, U32)
                if s == 0:
                    tt[NQ - 1, pl.ds(z0, TV - z0), :] = jnp.zeros((TV - z0, 2 * b), F32)
                    w0cp(0).wait()
                    g0 = _dot(X(foff[s], first[s]), w0[0])
                    w0cp(1).wait()
                    h_prev = _act(g0, _dot(X(foff[s], first[s]), w0[1]))
                else:
                    acc[:, pl.ds(foff[s - 1], first[s - 1])] = _down(w0[2], h_prev)
                    xs = X(foff[s], first[s])
                    h_prev = _act(_dot(xs, w0[0]), _dot(xs, w0[1]))
                for (s_, t0, t1, k0, k1) in xplan:
                    if s_ == s:
                        xtl = X(t0, t1 - t0, KM, KT).astype(F32)
                        for k in range(k0, k1):
                            xb[k, pl.ds(t0, t1 - t0), :] = jnp.broadcast_to(xtl[:, k:k + 1], (t1 - t0, 128))
                if s == NS - 1:
                    zz = zv[0]
                    prev = zz
                    for w in range(2):
                        for ci in range(NT):
                            def rp(rr, prev, w=w, ci=ci):
                                r16 = pl.multiple_of(rr * 16, 16)
                                r8 = pl.multiple_of(rr * 8, 8)
                                v = pltpu.bitcast(wm[w, 0, pl.ds(r16, 16), pl.ds(ci * 128, 128)], U32) | (prev & zz)
                                wpk[w, pl.ds(r8, 8), pl.ds(ci * 128, 128)] = v
                                return v
                            prev = lax.fori_loop(0, D // 16, rp, prev, unroll=True)
                    if fv_tiles:
                        tail_f32(0)
                        vpu_tail(range(fv_tiles), fv_rows, (fv_m,) * (fv_tiles * NQ))
                        assert fv_tiles == NT
                        tt[0, pl.ds(fv_rows, TV - fv_rows), pl.ds(0, b)] = _dot(
                            X(fv_rows, TV - fv_rows, KM, KT), wm[0, 0, pl.ds(KM, KT), :])
                    else:
                        tt[0, :, pl.ds(0, b)] = _dot(X(0, TV, KM, KT), wm[0, 0, pl.ds(KM, KT), :])
                    tt[0, :, pl.ds(b, b)] = _dot(X(0, TV, KM, KT), wm[1, 0, pl.ds(KM, KT), :])
                    acc[:, pl.ds(foff[s], first[s])] = _down(w0[2], h_prev)

            wmcp(2, 0).wait()

        def gu(r0, ts, tv, c0, nc):
            xm = X(r0, ts, 0, KM)
            g = _dot(xm, WP(0, 0, KM, c0, nc))
            u = _dot(xm, WP(1, 0, KM, c0, nc))
            pg, pu = [], []
            if tv:
                vg = tt[0, :, pl.ds(c0, nc)]
                vu = tt[0, :, pl.ds(b + c0, nc)]
                for q in range(1, NQ):
                    vg = vg + tt[q, :, pl.ds(c0, nc)]
                    vu = vu + tt[q, :, pl.ds(b + c0, nc)]
                pg.append(vg)
                pu.append(vu)
            xt_ = X(r0 + tv, ts - tv, KM, KT)
            pg.append(_dot(xt_, WP(0, KM, KT, c0, nc)))
            pu.append(_dot(xt_, WP(1, KM, KT, c0, nc)))
            return _act(g + jnp.concatenate(pg, axis=0), u + jnp.concatenate(pu, axis=0))

        def body(j, carry):
            for w in range(3):
                wmcp(w, j + 1).wait()
            tail_f32(j + 1)
            hs = [gu(moff[s], mid[s], TV if s == 0 else 0, 0, b) for s in range(len(mid))]
            vpu_tail(range(2 * NT), TV, mprof)
            for w in range(2):
                wpk[w] = pltpu.bitcast(wm[w, j + 1], U32)
            for s in range(len(mid)):
                acc[:, pl.ds(moff[s], mid[s])] += _down(wm[2, j], hs[s])
            return carry

        def last_block():
            c0 = b - c
            ocps = []

            def fin(s, h):
                sl = pl.ds(loff[s], last[s])
                nr = orows if s >= NL - nfin else 1
                val = ((acc[:, sl] + _down(wm[2, n, :, pl.ds(c0, c)], h)) * 0.5).astype(BF16)
                for r in range(nr):
                    rs = pl.ds(r * (D // nr), D // nr)
                    o_v[rs, sl] = val[r * (D // nr):(r + 1) * (D // nr)]
                    cp = ocp(s, r, nr)
                    cp.start()
                    ocps.append(cp)

            h_prev = None
            for s in range(NL):
                h = gu(loff[s], last[s], TV if s == 0 else 0, c0, c)
                if h_prev is not None:
                    fin(s - 1, h_prev)
                h_prev = h
            fin(NL - 1, h_prev)
            with scope("finalwait"):
                for cp in ocps:
                    cp.wait()

        if oneloop:
            def step(j, carry):
                @pl.when(j == 0)
                def _():
                    first_block()

                @pl.when(jnp.logical_and(j > 0, j <= n))
                def _():
                    with scope("iter"):
                        body(j - 1, 0)

                @pl.when(j == n + 1)
                def _():
                    with scope("last"):
                        last_block()
                return carry

            lax.fori_loop(0, n + 2, step, 0)
        else:
            first_block()
            with scope("loop"):
                lax.fori_loop(0, n, body, 0)
            last_block()

    def fn(x, w_gate, w_up, w_down):
        B, S, _ = x.shape
        xt = x.reshape(M, D).T
        wdt = w_down.T
        out_t = pl.pallas_call(
            kern,
            in_specs=[pl.BlockSpec(memory_space=pl.ANY)] * 4,
            out_specs=pl.BlockSpec(memory_space=pl.ANY),
            out_shape=jax.ShapeDtypeStruct((D, M), x.dtype),
            scratch_shapes=[
                pltpu.VMEM((D, M), BF16),
                pltpu.VMEM((M // 2, D), U32),
                pltpu.VMEM((3, D, a), BF16),
                pltpu.VMEM((3, n + 1, D, b), BF16),
                pltpu.VMEM((2, D // 2, b), U32),
                pltpu.VMEM((D, M), F32),
                pltpu.VMEM((D, M), BF16),
                pltpu.VMEM((KT, TV, 128), F32),
                pltpu.VMEM((KT, 2 * b), F32),
                pltpu.VMEM((NQ, TV, 2 * b), F32),
                pltpu.VMEM((2, 8, 128), U32),
                pltpu.SemaphoreType.DMA((NS + 3 + n + 2,)),
                pltpu.SemaphoreType.DMA((1,)),
            ],
            compiler_params=pltpu.CompilerParams(vmem_limit_bytes=110 * 1024 * 1024,
                                                 disable_semaphore_checks=True),
        )(xt, w_gate, w_up, wdt)
        return out_t.T.reshape(B, S, D)
    return fn


_impl = make()


@jax.jit
def pallas_standalone__geglu_ffn__prompt_kernel(
    x: jax.Array,
    w_gate: jax.Array,
    w_up: jax.Array,
    w_down: jax.Array,
):
    return _impl(x, w_gate, w_up, w_down)
```

```python
import jax
import jax.numpy as jnp
from jax import lax
import jax.experimental.pallas as pl
import jax.experimental.pallas.tpu as pltpu

F32 = jnp.float32
BF16 = jnp.bfloat16
U32 = jnp.uint32

D, M, F = 576, 2048, 4608
KM, KT = 512, 64
KQ = 16
NQ = KT // KQ
CA, CB, CC = 256, 512, 256
NB = (F - CA - CC) // CB
NT = CB // 128
FIRST = (256, 256, 768, 768)
MID = (640, 1408)
LAST = (640, 512, 384, 256, 256)
OROWS, NFIN = 4, 2
TV = 544
MPROF = (8,) * 4 + (7,) * 11 + (6,) * 17
Z0 = 200
XPLAN = ((1, 0, 512, 0, 8), (2, 512, TV, 0, 8), (2, 0, TV, 8, 48), (3, 0, TV, 48, 64))

assert CA + NB * CB + CC == F and CC <= CB
assert sum(FIRST) == M and sum(MID) == M and sum(LAST) == M
assert TV < MID[0] and TV < LAST[0] and TV % 16 == 0


def _offsets(sizes):
    return [sum(sizes[:i]) for i in range(len(sizes))]


FOFF, MOFF, LOFF = _offsets(FIRST), _offsets(MID), _offsets(LAST)
NS, NL = len(FIRST), len(LAST)


def _act(g, u):
    c = 0.7978845608028654
    inner = g * (c + (c * 0.044715) * (g * g))
    return ((g * (1.0 + jnp.tanh(inner))) * u).astype(BF16)


def _dot(a, b):
    return jnp.dot(a, b, preferred_element_type=F32)


def _down(wdt, h):
    return lax.dot_general(wdt, h, (((1,), (1,)), ((), ())), preferred_element_type=F32)


def _kernel(xt_hbm, wg_hbm, wu_hbm, wd_hbm, o_hbm,
            xt_v, x32, w0, wm, wpk, acc, o_v, xb, w32, tt, zv, isem, osem):
    whbm = (wg_hbm, wu_hbm, wd_hbm)

    def xcp(s):
        sl = pl.ds(FOFF[s], FIRST[s])
        return pltpu.make_async_copy(xt_hbm.at[:, sl], xt_v.at[:, sl], isem.at[s])

    def w0cp(w):
        return pltpu.make_async_copy(whbm[w].at[:, pl.ds(0, CA)], w0.at[w], isem.at[NS + w])

    def wmcp(w, j):
        if isinstance(j, int):
            off = min(CA + j * CB, F - CB)
        else:
            off = pl.multiple_of(jnp.minimum(CA + j * CB, F - CB), 128)
        sem = NS + 3 + j
        if isinstance(j, int) and j == 0 and w < 2:
            sem = NS + 3 + NB + 1
        return pltpu.make_async_copy(whbm[w].at[:, pl.ds(off, CB)], wm.at[w, j], isem.at[sem])

    def ocp(s, r, nr):
        sl = pl.ds(LOFF[s], LAST[s])
        rs = pl.ds(r * (D // nr), D // nr)
        return pltpu.make_async_copy(o_v.at[rs, sl], o_hbm.at[rs, sl], osem.at[0])

    def X(r0, nr, c0=0, nc=D):
        return pltpu.bitcast(x32[pl.ds(r0 // 2, nr // 2), pl.ds(c0, nc)], BF16)

    def WP(w, r0, nr, c0, nc):
        return pltpu.bitcast(wpk[w, pl.ds(r0 // 2, nr // 2), pl.ds(c0, nc)], BF16)

    def vpu_tail():
        never1 = zv[0] != 0
        never2 = zv[1] != 0
        zf = pltpu.bitcast(zv[0], F32)
        st = (zf, zf, zf, zf)
        for i in range(2 * NT):
            cs = pl.ds(i * 128, 128)
            for q in range(NQ):
                wr = [w32[pl.ds(q * KQ + kk, 1), cs] for kk in range(KQ)]

                def chain(t, st, q=q, m=MPROF[i * NQ + q], wr=wr, cs=cs):
                    f3, f2, f1, md = st
                    rows = pl.ds(pl.multiple_of(t * 8, 8), 8)
                    r = mv = None
                    for kk in range(KQ):
                        p = xb[q * KQ + kk, rows, :] * wr[kk]
                        if kk == 0:
                            r = jnp.where(never2, f3, jnp.where(never1, md, p))
                        else:
                            r = r + p
                        if kk + 1 == m:
                            mv = r
                    tt[q, rows, cs] = r
                    return (f2, f1, r, mv)

                st = lax.fori_loop(0, TV // 8, chain, st, unroll=True)

    def gu(r0, ts, tv, c0, nc):
        xm = X(r0, ts, 0, KM)
        g = _dot(xm, WP(0, 0, KM, c0, nc))
        u = _dot(xm, WP(1, 0, KM, c0, nc))
        pg, pu = [], []
        if tv:
            vg = tt[0, :, pl.ds(c0, nc)]
            vu = tt[0, :, pl.ds(CB + c0, nc)]
            for q in range(1, NQ):
                vg = vg + tt[q, :, pl.ds(c0, nc)]
                vu = vu + tt[q, :, pl.ds(CB + c0, nc)]
            pg.append(vg)
            pu.append(vu)
        xt_ = X(r0 + tv, ts - tv, KM, KT)
        pg.append(_dot(xt_, WP(0, KM, KT, c0, nc)))
        pu.append(_dot(xt_, WP(1, KM, KT, c0, nc)))
        return _act(g + jnp.concatenate(pg, axis=0), u + jnp.concatenate(pu, axis=0))

    def first_block():
        h_prev = None
        for s in range(NS):
            sl = pl.ds(FOFF[s], FIRST[s])
            xcp(s).wait()
            if s == 1:
                w0cp(2).wait()
            if s == NS - 1:
                wmcp(0, 0).wait()
                wmcp(1, 0).wait()
            x32[pl.ds(FOFF[s] // 2, FIRST[s] // 2), :] = pltpu.bitcast(xt_v[:, sl].T, U32)
            if s == 0:
                tt[NQ - 1, pl.ds(Z0, TV - Z0), :] = jnp.zeros((TV - Z0, 2 * CB), F32)
                w0cp(0).wait()
                g0 = _dot(X(FOFF[s], FIRST[s]), w0[0])
                w0cp(1).wait()
                h_prev = _act(g0, _dot(X(FOFF[s], FIRST[s]), w0[1]))
            else:
                acc[:, pl.ds(FOFF[s - 1], FIRST[s - 1])] = _down(w0[2], h_prev)
                xs = X(FOFF[s], FIRST[s])
                h_prev = _act(_dot(xs, w0[0]), _dot(xs, w0[1]))
            for (s_, t0, t1, k0, k1) in XPLAN:
                if s_ == s:
                    xtl = X(t0, t1 - t0, KM, KT).astype(F32)
                    for k in range(k0, k1):
                        xb[k, pl.ds(t0, t1 - t0), :] = jnp.broadcast_to(xtl[:, k:k + 1], (t1 - t0, 128))
            if s == NS - 1:
                zz = zv[0]
                prev = zz
                for w in range(2):
                    for ci in range(NT):
                        def rp(rr, prev, w=w, ci=ci):
                            r16 = pl.multiple_of(rr * 16, 16)
                            r8 = pl.multiple_of(rr * 8, 8)
                            v = pltpu.bitcast(wm[w, 0, pl.ds(r16, 16), pl.ds(ci * 128, 128)], U32) | (prev & zz)
                            wpk[w, pl.ds(r8, 8), pl.ds(ci * 128, 128)] = v
                            return v
                        prev = lax.fori_loop(0, D // 16, rp, prev, unroll=True)
                xtl = X(0, TV, KM, KT)
                tt[0, :, pl.ds(0, CB)] = _dot(xtl, wm[0, 0, pl.ds(KM, KT), :])
                tt[0, :, pl.ds(CB, CB)] = _dot(xtl, wm[1, 0, pl.ds(KM, KT), :])
                acc[:, pl.ds(FOFF[s], FIRST[s])] = _down(w0[2], h_prev)
        wmcp(2, 0).wait()

    def body(j, carry):
        for w in range(3):
            wmcp(w, j + 1).wait()
        w32[:, pl.ds(0, CB)] = wm[0, j + 1, pl.ds(KM, KT), :].astype(F32)
        w32[:, pl.ds(CB, CB)] = wm[1, j + 1, pl.ds(KM, KT), :].astype(F32)
        hs = [gu(MOFF[s], MID[s], TV if s == 0 else 0, 0, CB) for s in range(len(MID))]
        vpu_tail()
        for w in range(2):
            wpk[w] = pltpu.bitcast(wm[w, j + 1], U32)
        for s in range(len(MID)):
            acc[:, pl.ds(MOFF[s], MID[s])] += _down(wm[2, j], hs[s])
        return carry

    def last_block():
        c0 = CB - CC
        ocps = []

        def fin(s, h):
            sl = pl.ds(LOFF[s], LAST[s])
            nr = OROWS if s >= NL - NFIN else 1
            val = ((acc[:, sl] + _down(wm[2, NB, :, pl.ds(c0, CC)], h)) * 0.5).astype(BF16)
            for r in range(nr):
                rs = pl.ds(r * (D // nr), D // nr)
                o_v[rs, sl] = val[r * (D // nr):(r + 1) * (D // nr)]
                cp = ocp(s, r, nr)
                cp.start()
                ocps.append(cp)

        h_prev = None
        for s in range(NL):
            h = gu(LOFF[s], LAST[s], TV if s == 0 else 0, c0, CC)
            if h_prev is not None:
                fin(s - 1, h_prev)
            h_prev = h
        fin(NL - 1, h_prev)
        for cp in ocps:
            cp.wait()

    xcp(0).start()
    w0cp(0).start()
    w0cp(1).start()
    xcp(1).start()
    w0cp(2).start()
    for s in range(2, NS - 1):
        xcp(s).start()
    wmcp(0, 0).start()
    wmcp(1, 0).start()
    xcp(NS - 1).start()
    wmcp(2, 0).start(priority=1)
    for j in range(1, NB + 1):
        for w in range(3):
            wmcp(w, j).start(priority=1)

    zv[...] = jnp.zeros(zv.shape, U32)
    for q in range(1, NQ - 1):
        tt[q] = jnp.zeros((TV, 2 * CB), F32)
    tt[NQ - 1, pl.ds(0, Z0), :] = jnp.zeros((Z0, 2 * CB), F32)

    def phase(p, carry):
        @pl.when(p == 0)
        def _():
            first_block()

        @pl.when(p == 1)
        def _():
            lax.fori_loop(0, NB, body, 0)

        @pl.when(p == 2)
        def _():
            last_block()

        return carry

    lax.fori_loop(0, 3, phase, 0)


@jax.jit
def pallas_standalone__geglu_ffn__prompt_kernel(
    x: jax.Array,
    w_gate: jax.Array,
    w_up: jax.Array,
    w_down: jax.Array,
):
    B, S, _ = x.shape
    assert (B * S, x.shape[2]) == (M, D) and w_gate.shape == (D, F) and w_down.shape == (F, D)
    out_t = pl.pallas_call(
        _kernel,
        in_specs=[pl.BlockSpec(memory_space=pl.ANY)] * 4,
        out_specs=pl.BlockSpec(memory_space=pl.ANY),
        out_shape=jax.ShapeDtypeStruct((D, M), x.dtype),
        scratch_shapes=[
            pltpu.VMEM((D, M), BF16),
            pltpu.VMEM((M // 2, D), U32),
            pltpu.VMEM((3, D, CA), BF16),
            pltpu.VMEM((3, NB + 1, D, CB), BF16),
            pltpu.VMEM((2, D // 2, CB), U32),
            pltpu.VMEM((D, M), F32),
            pltpu.VMEM((D, M), BF16),
            pltpu.VMEM((KT, TV, 128), F32),
            pltpu.VMEM((KT, 2 * CB), F32),
            pltpu.VMEM((NQ, TV, 2 * CB), F32),
            pltpu.VMEM((2, 8, 128), U32),
            pltpu.SemaphoreType.DMA((NS + 3 + NB + 2,)),
            pltpu.SemaphoreType.DMA((1,)),
        ],
        compiler_params=pltpu.CompilerParams(
            vmem_limit_bytes=110 * 1024 * 1024,
            disable_semaphore_checks=True,
        ),
    )(x.reshape(M, D).T, w_gate, w_up, w_down.T)
    return out_t.T.reshape(B, S, D)
```

```python
import jax
import jax.numpy as jnp
from jax import lax
import jax.experimental.pallas as pl
import jax.experimental.pallas.tpu as pltpu

F32 = jnp.float32
BF16 = jnp.bfloat16
U32 = jnp.uint32

D, M, F = 576, 2048, 4608
KM, KT = 512, 64
KQ = 16
NQ = KT // KQ
CA, CB, CC = 256, 512, 256
NB = (F - CA - CC) // CB
NT = CB // 128
FIRST = (256, 256, 768, 768)
MID = (640, 1408)
LAST = (640, 512, 384, 256, 256)
OROWS, NFIN = 4, 2
TV = 544
MPROF = (8,) * 3 + (7,) * 12 + (6,) * 17
Z0 = 200
XPLAN = ((1, 0, 512, 0, 8), (2, 512, TV, 0, 8), (2, 0, TV, 8, 48), (3, 0, TV, 48, 64))

assert CA + NB * CB + CC == F and CC <= CB
assert sum(FIRST) == M and sum(MID) == M and sum(LAST) == M
assert TV < MID[0] and TV < LAST[0] and TV % 16 == 0


def _offsets(sizes):
    return [sum(sizes[:i]) for i in range(len(sizes))]


FOFF, MOFF, LOFF = _offsets(FIRST), _offsets(MID), _offsets(LAST)
NS, NL = len(FIRST), len(LAST)


def _act(g, u):
    c = 0.7978845608028654
    inner = g * (c + (c * 0.044715) * (g * g))
    return ((g * (1.0 + jnp.tanh(inner))) * u).astype(BF16)


def _dot(a, b):
    return jnp.dot(a, b, preferred_element_type=F32)


def _down(wdt, h):
    return lax.dot_general(wdt, h, (((1,), (1,)), ((), ())), preferred_element_type=F32)


def _kernel(xt_hbm, wg_hbm, wu_hbm, wd_hbm, o_hbm,
            xt_v, x32, w0, wm, wpk, acc, o_v, xb, w32, tt, zv, isem, osem):
    whbm = (wg_hbm, wu_hbm, wd_hbm)

    def xcp(s):
        sl = pl.ds(FOFF[s], FIRST[s])
        return pltpu.make_async_copy(xt_hbm.at[:, sl], xt_v.at[:, sl], isem.at[s])

    def w0cp(w):
        return pltpu.make_async_copy(whbm[w].at[:, pl.ds(0, CA)], w0.at[w], isem.at[NS + w])

    def wmcp(w, j):
        if isinstance(j, int):
            off = min(CA + j * CB, F - CB)
        else:
            off = pl.multiple_of(jnp.minimum(CA + j * CB, F - CB), 128)
        sem = NS + 3 + j
        if isinstance(j, int) and j == 0 and w < 2:
            sem = NS + 3 + NB + 1
        return pltpu.make_async_copy(whbm[w].at[:, pl.ds(off, CB)], wm.at[w, j], isem.at[sem])

    def ocp(s, r, nr):
        sl = pl.ds(LOFF[s], LAST[s])
        rs = pl.ds(r * (D // nr), D // nr)
        return pltpu.make_async_copy(o_v.at[rs, sl], o_hbm.at[rs, sl], osem.at[0])

    def X(r0, nr, c0=0, nc=D):
        return pltpu.bitcast(x32[pl.ds(r0 // 2, nr // 2), pl.ds(c0, nc)], BF16)

    def WP(w, r0, nr, c0, nc):
        return pltpu.bitcast(wpk[w, pl.ds(r0 // 2, nr // 2), pl.ds(c0, nc)], BF16)

    def vpu_tail():
        never1 = zv[0] != 0
        never2 = zv[1] != 0
        zf = pltpu.bitcast(zv[0], F32)
        st = (zf, zf, zf, zf)
        for i in range(2 * NT):
            cs = pl.ds(i * 128, 128)
            for q in range(NQ):
                wr = [w32[pl.ds(q * KQ + kk, 1), cs] for kk in range(KQ)]

                def chain(t, st, q=q, m=MPROF[i * NQ + q], wr=wr, cs=cs):
                    f3, f2, f1, md = st
                    rows = pl.ds(pl.multiple_of(t * 8, 8), 8)
                    xq = xb[pl.ds(q * KQ, KQ), rows, :]
                    r = mv = None
                    for kk in range(KQ):
                        p = xq[kk] * wr[kk]
                        if kk == 0:
                            r = jnp.where(never2, f3, jnp.where(never1, md, p))
                        else:
                            r = r + p
                        if kk + 1 == m:
                            mv = r
                    tt[q, rows, cs] = r
                    return (f2, f1, r, mv)

                st = lax.fori_loop(0, TV // 8, chain, st, unroll=True)

    def gu(r0, ts, tv, c0, nc):
        xm = X(r0, ts, 0, KM)
        g = _dot(xm, WP(0, 0, KM, c0, nc))
        u = _dot(xm, WP(1, 0, KM, c0, nc))
        pg, pu = [], []
        if tv:
            vg = tt[0, :, pl.ds(c0, nc)]
            vu = tt[0, :, pl.ds(CB + c0, nc)]
            for q in range(1, NQ):
                vg = vg + tt[q, :, pl.ds(c0, nc)]
                vu = vu + tt[q, :, pl.ds(CB + c0, nc)]
            pg.append(vg)
            pu.append(vu)
        xt_ = X(r0 + tv, ts - tv, KM, KT)
        pg.append(_dot(xt_, WP(0, KM, KT, c0, nc)))
        pu.append(_dot(xt_, WP(1, KM, KT, c0, nc)))
        return _act(g + jnp.concatenate(pg, axis=0), u + jnp.concatenate(pu, axis=0))

    def first_block():
        h_prev = None
        for s in range(NS):
            sl = pl.ds(FOFF[s], FIRST[s])
            xcp(s).wait()
            if s == 1:
                w0cp(2).wait()
            if s == NS - 1:
                wmcp(0, 0).wait()
                wmcp(1, 0).wait()
            x32[pl.ds(FOFF[s] // 2, FIRST[s] // 2), :] = pltpu.bitcast(xt_v[:, sl].T, U32)
            if s == 0:
                tt[NQ - 1, pl.ds(Z0, TV - Z0), :] = jnp.zeros((TV - Z0, 2 * CB), F32)
                w0cp(0).wait()
                g0 = _dot(X(FOFF[s], FIRST[s]), w0[0])
                w0cp(1).wait()
                h_prev = _act(g0, _dot(X(FOFF[s], FIRST[s]), w0[1]))
            else:
                acc[:, pl.ds(FOFF[s - 1], FIRST[s - 1])] = _down(w0[2], h_prev)
                xs = X(FOFF[s], FIRST[s])
                h_prev = _act(_dot(xs, w0[0]), _dot(xs, w0[1]))
            for (s_, t0, t1, k0, k1) in XPLAN:
                if s_ == s:
                    xtl = X(t0, t1 - t0, KM, KT).astype(F32)
                    for k in range(k0, k1):
                        xb[k, pl.ds(t0, t1 - t0), :] = jnp.broadcast_to(xtl[:, k:k + 1], (t1 - t0, 128))
            if s == NS - 1:
                zz = zv[0]
                prev = zz
                for w in range(2):
                    for ci in range(NT):
                        def rp(rr, prev, w=w, ci=ci):
                            r16 = pl.multiple_of(rr * 16, 16)
                            r8 = pl.multiple_of(rr * 8, 8)
                            v = pltpu.bitcast(wm[w, 0, pl.ds(r16, 16), pl.ds(ci * 128, 128)], U32) | (prev & zz)
                            wpk[w, pl.ds(r8, 8), pl.ds(ci * 128, 128)] = v
                            return v
                        prev = lax.fori_loop(0, D // 16, rp, prev, unroll=True)
                xtl = X(0, TV, KM, KT)
                tt[0, :, pl.ds(0, CB)] = _dot(xtl, wm[0, 0, pl.ds(KM, KT), :])
                tt[0, :, pl.ds(CB, CB)] = _dot(xtl, wm[1, 0, pl.ds(KM, KT), :])
                acc[:, pl.ds(FOFF[s], FIRST[s])] = _down(w0[2], h_prev)
        wmcp(2, 0).wait()

    def body(j, carry):
        for w in range(3):
            wmcp(w, j + 1).wait()
        w32[:, pl.ds(0, CB)] = wm[0, j + 1, pl.ds(KM, KT), :].astype(F32)
        w32[:, pl.ds(CB, CB)] = wm[1, j + 1, pl.ds(KM, KT), :].astype(F32)
        hs = [gu(MOFF[s], MID[s], TV if s == 0 else 0, 0, CB) for s in range(len(MID))]
        vpu_tail()
        for w in range(2):
            wpk[w] = pltpu.bitcast(wm[w, j + 1], U32)
        for s in range(len(MID)):
            acc[:, pl.ds(MOFF[s], MID[s])] += _down(wm[2, j], hs[s])
        return carry

    def last_block():
        c0 = CB - CC
        ocps = []

        def fin(s, h):
            sl = pl.ds(LOFF[s], LAST[s])
            nr = OROWS if s >= NL - NFIN else 1
            val = ((acc[:, sl] + _down(wm[2, NB, :, pl.ds(c0, CC)], h)) * 0.5).astype(BF16)
            for r in range(nr):
                rs = pl.ds(r * (D // nr), D // nr)
                o_v[rs, sl] = val[r * (D // nr):(r + 1) * (D // nr)]
                cp = ocp(s, r, nr)
                cp.start()
                ocps.append(cp)

        h_prev = None
        for s in range(NL):
            h = gu(LOFF[s], LAST[s], TV if s == 0 else 0, c0, CC)
            if h_prev is not None:
                fin(s - 1, h_prev)
            h_prev = h
        fin(NL - 1, h_prev)
        for cp in ocps:
            cp.wait()

    def prologue():
        xcp(0).start()
        w0cp(0).start()
        w0cp(1).start()
        xcp(1).start()
        w0cp(2).start()
        for s in range(2, NS - 1):
            xcp(s).start()
        wmcp(0, 0).start()
        wmcp(1, 0).start()
        xcp(NS - 1).start()
        wmcp(2, 0).start(priority=1)
        for j in range(1, NB + 1):
            for w in range(3):
                wmcp(w, j).start(priority=1)

        zv[...] = jnp.zeros(zv.shape, U32)
        for q in range(1, NQ - 1):
            tt[q] = jnp.zeros((TV, 2 * CB), F32)
        tt[NQ - 1, pl.ds(0, Z0), :] = jnp.zeros((Z0, 2 * CB), F32)

    p = pl.program_id(0)

    @pl.when(p == 0)
    def _():
        prologue()
        first_block()

    @pl.when(p == 1)
    def _():
        lax.fori_loop(0, NB, body, 0)

    @pl.when(p == 2)
    def _():
        last_block()


@jax.jit
def pallas_standalone__geglu_ffn__prompt_kernel(
    x: jax.Array,
    w_gate: jax.Array,
    w_up: jax.Array,
    w_down: jax.Array,
):
    B, S, _ = x.shape
    assert (B * S, x.shape[2]) == (M, D) and w_gate.shape == (D, F) and w_down.shape == (F, D)
    out_t = pl.pallas_call(
        _kernel,
        grid=(3,),
        in_specs=[pl.BlockSpec(memory_space=pl.ANY)] * 4,
        out_specs=pl.BlockSpec(memory_space=pl.ANY),
        out_shape=jax.ShapeDtypeStruct((D, M), x.dtype),
        scratch_shapes=[
            pltpu.VMEM((D, M), BF16),
            pltpu.VMEM((M // 2, D), U32),
            pltpu.VMEM((3, D, CA), BF16),
            pltpu.VMEM((3, NB + 1, D, CB), BF16),
            pltpu.VMEM((2, D // 2, CB), U32),
            pltpu.VMEM((D, M), F32),
            pltpu.VMEM((D, M), BF16),
            pltpu.VMEM((KT, TV, 128), F32),
            pltpu.VMEM((KT, 2 * CB), F32),
            pltpu.VMEM((NQ, TV, 2 * CB), F32),
            pltpu.VMEM((2, 8, 128), U32),
            pltpu.SemaphoreType.DMA((NS + 3 + NB + 2,)),
            pltpu.SemaphoreType.DMA((1,)),
        ],
        compiler_params=pltpu.CompilerParams(
            dimension_semantics=("arbitrary",),
            vmem_limit_bytes=110 * 1024 * 1024,
            disable_semaphore_checks=True,
        ),
    )(x.reshape(M, D).T, w_gate, w_up, w_down.T)
    return out_t.T.reshape(B, S, D)
```

```python
import jax
import jax.numpy as jnp
from jax import lax
import jax.experimental.pallas as pl
import jax.experimental.pallas.tpu as pltpu

F32 = jnp.float32
BF16 = jnp.bfloat16
U32 = jnp.uint32

D, M, F = 576, 2048, 4608
KM, KT = 512, 64
KQ = 16
NQ = KT // KQ
CA, CB, CC = 256, 512, 256
NB = (F - CA - CC) // CB
NT = CB // 128
FIRST = (256, 256, 768, 768)
MID = (640, 1408)
LAST = (640, 512, 384, 256, 256)
OROWS, NFIN = 12, 2
TV = 544
MPROF = (8,) * 4 + (7,) * 11 + (6,) * 17
Z0 = 200
XPLAN = ((1, 0, 512, 0, 8), (2, 512, TV, 0, 8), (2, 0, TV, 8, 48), (3, 0, TV, 48, 64))

assert CA + NB * CB + CC == F and CC <= CB
assert sum(FIRST) == M and sum(MID) == M and sum(LAST) == M
assert TV < MID[0] and TV < LAST[0] and TV % 16 == 0


def _offsets(sizes):
    return [sum(sizes[:i]) for i in range(len(sizes))]


FOFF, MOFF, LOFF = _offsets(FIRST), _offsets(MID), _offsets(LAST)
NS, NL = len(FIRST), len(LAST)


def _act(g, u):
    c = 0.7978845608028654
    inner = g * (c + (c * 0.044715) * (g * g))
    return ((g * (1.0 + jnp.tanh(inner))) * u).astype(BF16)


def _dot(a, b):
    return jnp.dot(a, b, preferred_element_type=F32)


def _down(wdt, h):
    return lax.dot_general(wdt, h, (((1,), (1,)), ((), ())), preferred_element_type=F32)


def _kernel(xt_hbm, wg_hbm, wu_hbm, wd_hbm, o_hbm,
            xt_v, x32, w0, wm, wpk, acc, o_v, xb, w32, tt, zv, isem, osem):
    whbm = (wg_hbm, wu_hbm, wd_hbm)

    def xcp(s):
        sl = pl.ds(FOFF[s], FIRST[s])
        return pltpu.make_async_copy(xt_hbm.at[:, sl], xt_v.at[:, sl], isem.at[s])

    def w0cp(w):
        return pltpu.make_async_copy(whbm[w].at[:, pl.ds(0, CA)], w0.at[w], isem.at[NS + w])

    def wmcp(w, j):
        if isinstance(j, int):
            off = min(CA + j * CB, F - CB)
        else:
            off = pl.multiple_of(jnp.minimum(CA + j * CB, F - CB), 128)
        sem = NS + 3 + j
        if isinstance(j, int) and j == 0 and w < 2:
            sem = NS + 3 + NB + 1
        return pltpu.make_async_copy(whbm[w].at[:, pl.ds(off, CB)], wm.at[w, j], isem.at[sem])

    def ocp(s, r, nr):
        sl = pl.ds(LOFF[s], LAST[s])
        rs = pl.ds(r * (D // nr), D // nr)
        return pltpu.make_async_copy(o_v.at[rs, sl], o_hbm.at[rs, sl], osem.at[0])

    def X(r0, nr, c0=0, nc=D):
        return pltpu.bitcast(x32[pl.ds(r0 // 2, nr // 2), pl.ds(c0, nc)], BF16)

    def WP(w, r0, nr, c0, nc):
        return pltpu.bitcast(wpk[w, pl.ds(r0 // 2, nr // 2), pl.ds(c0, nc)], BF16)

    def vpu_tail():
        never1 = zv[0] != 0
        never2 = zv[1] != 0
        zf = pltpu.bitcast(zv[0], F32)
        st = (zf, zf, zf, zf)
        for i in range(2 * NT):
            cs = pl.ds(i * 128, 128)
            for q in range(NQ):
                wr = [w32[pl.ds(q * KQ + kk, 1), cs] for kk in range(KQ)]

                def chain(t, st, q=q, m=MPROF[i * NQ + q], wr=wr, cs=cs):
                    f3, f2, f1, md = st
                    rows = pl.ds(pl.multiple_of(t * 8, 8), 8)
                    r = mv = None
                    for kk in range(KQ):
                        p = xb[q * KQ + kk, rows, :] * wr[kk]
                        if kk == 0:
                            r = jnp.where(never2, f3, jnp.where(never1, md, p))
                        else:
                            r = r + p
                        if kk + 1 == m:
                            mv = r
                    tt[q, rows, cs] = r
                    return (f2, f1, r, mv)

                st = lax.fori_loop(0, TV // 8, chain, st, unroll=True)

    def gu(r0, ts, tv, c0, nc):
        xm = X(r0, ts, 0, KM)
        g = _dot(xm, WP(0, 0, KM, c0, nc))
        u = _dot(xm, WP(1, 0, KM, c0, nc))
        pg, pu = [], []
        if tv:
            vg = tt[0, :, pl.ds(c0, nc)]
            vu = tt[0, :, pl.ds(CB + c0, nc)]
            for q in range(1, NQ):
                vg = vg + tt[q, :, pl.ds(c0, nc)]
                vu = vu + tt[q, :, pl.ds(CB + c0, nc)]
            pg.append(vg)
            pu.append(vu)
        xt_ = X(r0 + tv, ts - tv, KM, KT)
        pg.append(_dot(xt_, WP(0, KM, KT, c0, nc)))
        pu.append(_dot(xt_, WP(1, KM, KT, c0, nc)))
        return _act(g + jnp.concatenate(pg, axis=0), u + jnp.concatenate(pu, axis=0))

    def first_block():
        h_prev = None
        for s in range(NS):
            sl = pl.ds(FOFF[s], FIRST[s])
            xcp(s).wait()
            if s == 1:
                w0cp(2).wait()
            if s == NS - 1:
                wmcp(0, 0).wait()
                wmcp(1, 0).wait()
            x32[pl.ds(FOFF[s] // 2, FIRST[s] // 2), :] = pltpu.bitcast(xt_v[:, sl].T, U32)
            if s == 0:
                tt[NQ - 1, pl.ds(Z0, TV - Z0), :] = jnp.zeros((TV - Z0, 2 * CB), F32)
                w0cp(0).wait()
                g0 = _dot(X(FOFF[s], FIRST[s]), w0[0])
                w0cp(1).wait()
                h_prev = _act(g0, _dot(X(FOFF[s], FIRST[s]), w0[1]))
            else:
                acc[:, pl.ds(FOFF[s - 1], FIRST[s - 1])] = _down(w0[2], h_prev)
                xs = X(FOFF[s], FIRST[s])
                h_prev = _act(_dot(xs, w0[0]), _dot(xs, w0[1]))
            for (s_, t0, t1, k0, k1) in XPLAN:
                if s_ == s:
                    xtl = X(t0, t1 - t0, KM, KT).astype(F32)
                    for k in range(k0, k1):
                        xb[k, pl.ds(t0, t1 - t0), :] = jnp.broadcast_to(xtl[:, k:k + 1], (t1 - t0, 128))
            if s == NS - 1:
                zz = zv[0]
                prev = zz
                for w in range(2):
                    for ci in range(NT):
                        def rp(rr, prev, w=w, ci=ci):
                            r16 = pl.multiple_of(rr * 16, 16)
                            r8 = pl.multiple_of(rr * 8, 8)
                            v = pltpu.bitcast(wm[w, 0, pl.ds(r16, 16), pl.ds(ci * 128, 128)], U32) | (prev & zz)
                            wpk[w, pl.ds(r8, 8), pl.ds(ci * 128, 128)] = v
                            return v
                        prev = lax.fori_loop(0, D // 16, rp, prev, unroll=True)
                xtl = X(0, TV, KM, KT)
                tt[0, :, pl.ds(0, CB)] = _dot(xtl, wm[0, 0, pl.ds(KM, KT), :])
                tt[0, :, pl.ds(CB, CB)] = _dot(xtl, wm[1, 0, pl.ds(KM, KT), :])
                acc[:, pl.ds(FOFF[s], FIRST[s])] = _down(w0[2], h_prev)
        wmcp(2, 0).wait()

    def body(j, carry):
        for w in range(3):
            wmcp(w, j + 1).wait()
        w32[:, pl.ds(0, CB)] = wm[0, j + 1, pl.ds(KM, KT), :].astype(F32)
        w32[:, pl.ds(CB, CB)] = wm[1, j + 1, pl.ds(KM, KT), :].astype(F32)
        hs = [gu(MOFF[s], MID[s], TV if s == 0 else 0, 0, CB) for s in range(len(MID))]
        vpu_tail()
        for w in range(2):
            wpk[w] = pltpu.bitcast(wm[w, j + 1], U32)
        for s in range(len(MID)):
            acc[:, pl.ds(MOFF[s], MID[s])] += _down(wm[2, j], hs[s])
        return carry

    def last_block():
        c0 = CB - CC
        ocps = []

        def fin(s, h):
            sl = pl.ds(LOFF[s], LAST[s])
            nr = OROWS if s >= NL - NFIN else 1
            val = ((acc[:, sl] + _down(wm[2, NB, :, pl.ds(c0, CC)], h)) * 0.5).astype(BF16)
            for r in range(nr):
                rs = pl.ds(r * (D // nr), D // nr)
                o_v[rs, sl] = val[r * (D // nr):(r + 1) * (D // nr)]
                cp = ocp(s, r, nr)
                cp.start()
                ocps.append(cp)

        h_prev = None
        for s in range(NL):
            h = gu(LOFF[s], LAST[s], TV if s == 0 else 0, c0, CC)
            if h_prev is not None:
                fin(s - 1, h_prev)
            h_prev = h
        fin(NL - 1, h_prev)
        for cp in ocps:
            cp.wait()

    def prologue():
        xcp(0).start()
        w0cp(0).start()
        w0cp(1).start()
        xcp(1).start()
        w0cp(2).start()
        for s in range(2, NS - 1):
            xcp(s).start()
        wmcp(0, 0).start()
        wmcp(1, 0).start()
        xcp(NS - 1).start()
        wmcp(2, 0).start(priority=1)
        for j in range(1, NB + 1):
            for w in range(3):
                wmcp(w, j).start(priority=1)

        zv[...] = jnp.zeros(zv.shape, U32)
        for q in range(1, NQ - 1):
            tt[q] = jnp.zeros((TV, 2 * CB), F32)
        tt[NQ - 1, pl.ds(0, Z0), :] = jnp.zeros((Z0, 2 * CB), F32)

    p = pl.program_id(0)

    @pl.when(p == 0)
    def _():
        prologue()
        first_block()

    @pl.when(p == 1)
    def _():
        lax.fori_loop(0, NB, body, 0)

    @pl.when(p == 2)
    def _():
        last_block()


@jax.jit
def pallas_standalone__geglu_ffn__prompt_kernel(
    x: jax.Array,
    w_gate: jax.Array,
    w_up: jax.Array,
    w_down: jax.Array,
):
    B, S, _ = x.shape
    assert (B * S, x.shape[2]) == (M, D) and w_gate.shape == (D, F) and w_down.shape == (F, D)
    out_t = pl.pallas_call(
        _kernel,
        grid=(3,),
        in_specs=[pl.BlockSpec(memory_space=pl.ANY)] * 4,
        out_specs=pl.BlockSpec(memory_space=pl.ANY),
        out_shape=jax.ShapeDtypeStruct((D, M), x.dtype),
        scratch_shapes=[
            pltpu.VMEM((D, M), BF16),
            pltpu.VMEM((M // 2, D), U32),
            pltpu.VMEM((3, D, CA), BF16),
            pltpu.VMEM((3, NB + 1, D, CB), BF16),
            pltpu.VMEM((2, D // 2, CB), U32),
            pltpu.VMEM((D, M), F32),
            pltpu.VMEM((D, M), BF16),
            pltpu.VMEM((KT, TV, 128), F32),
            pltpu.VMEM((KT, 2 * CB), F32),
            pltpu.VMEM((NQ, TV, 2 * CB), F32),
            pltpu.VMEM((2, 8, 128), U32),
            pltpu.SemaphoreType.DMA((NS + 3 + NB + 2,)),
            pltpu.SemaphoreType.DMA((1,)),
        ],
        compiler_params=pltpu.CompilerParams(
            dimension_semantics=("arbitrary",),
            vmem_limit_bytes=110 * 1024 * 1024,
            disable_semaphore_checks=True,
        ),
    )(x.reshape(M, D).T, w_gate, w_up, w_down.T)
    return out_t.T.reshape(B, S, D)
```
